```python
import jax
import jax.numpy as jnp

def _softmax(x, axis=-1):
    return jax.nn.softmax(x, axis=axis)

def _gelu(x):
    return jax.nn.gelu(x, approximate=True)

def _silu(x):
    return jax.nn.silu(x)

def _sigmoid(x):
    return jax.nn.sigmoid(x)

def _layernorm(x, axis=-1, eps=1e-05):
    m = jnp.mean(x, axis=axis, keepdims=True)
    v = jnp.var(x, axis=axis, keepdims=True)
    return (x - m) / jnp.sqrt(v + eps)

def _scatter_add(tgt, idx, src, axis=0):
    return tgt.at[idx].add(src)

def _segment_sum(src, seg, n):
    return jax.ops.segment_sum(src, seg, n)

class _Rng:

    def __init__(self, key):
        self._k = key

    def _next(self):
        self._k, sub = jax.random.split(self._k)
        return sub

    def normal(self, shape):
        return jax.random.normal(self._next(), shape, dtype=jnp.bfloat16)

    def randint(self, lo, hi, shape):
        return jax.random.randint(self._next(), shape, lo, hi, dtype=jnp.int32)

    def uniform(self, shape, lo=0.0, hi=1.0):
        return jax.random.uniform(self._next(), shape, jnp.bfloat16, lo, hi)

    def permutation(self, n):
        return jax.random.permutation(self._next(), n)
kernel_name = 'recurrent_scan__memory_aug_recurrent_mem_tr__mixer_s_mlp__prompt'

def setup_inputs():
    _rng = _Rng(jax.random.key(int.from_bytes(__import__("os").urandom(4), "little")))
    _w = lambda a: (lambda t: t.astype(jnp.bfloat16) if jnp.issubdtype(t.dtype, jnp.floating) else t)(jnp.asarray(a))

    def _A_setup():
        B, S, Dm = (1, 2048, 1024)
        H, Dh = (32, 128)
        M, seg = (8, 32)
        seg = min(seg, S)
        S = S // seg * seg
        return {'x': _w((lambda *s: _rng.normal(s) * 0.05)(B, S, Dm)), 'mem0': _w((lambda *s: _rng.normal(s) * 0.05)(B, M, Dm)), 'Wq': _w((lambda *s: _rng.normal(s) * 0.05)(Dm, H, Dh) * Dm ** (-0.5)), 'Wk': _w((lambda *s: _rng.normal(s) * 0.05)(Dm, H, Dh) * Dm ** (-0.5)), 'Wv': _w((lambda *s: _rng.normal(s) * 0.05)(Dm, H, Dh) * Dm ** (-0.5)), 'Wo': _w((lambda *s: _rng.normal(s) * 0.05)(H, Dh, Dm) * (H * Dh) ** (-0.5)), 'seg_len': seg}
    _A_in = _A_setup()

    def _B_setup():
        B, S, D, F = (1, 2048, 1024, 3584)
        return {'x': _w((lambda *s: _rng.normal(s) * 0.05)(B, S, D)), 'w1': _w((lambda *s: _rng.normal(s) * 0.05)(D, D) * D ** (-0.5)), 'w2': _w((lambda *s: _rng.normal(s) * 0.05)(D, D) * D ** (-0.5)), 'w3': _w((lambda *s: _rng.normal(s) * 0.05)(D, F) * D ** (-0.5)), 'w4': _w((lambda *s: _rng.normal(s) * 0.05)(F, D) * F ** (-0.5))}
    _B_in = _B_setup()
    return {'A_x': _A_in['x'], 'A_mem0': _A_in['mem0'], 'A_Wq': _A_in['Wq'], 'A_Wk': _A_in['Wk'], 'A_Wv': _A_in['Wv'], 'A_Wo': _A_in['Wo'], 'A_seg_len': _A_in['seg_len'], 'B_x': _B_in['x'], 'B_w1': _B_in['w1'], 'B_w2': _B_in['w2'], 'B_w3': _B_in['w3'], 'B_w4': _B_in['w4']}

def reference(A_x, A_mem0, A_Wq, A_Wk, A_Wv, A_Wo, A_seg_len, B_x, B_w1, B_w2, B_w3, B_w4):

    def _A_ref(x, mem0, Wq, Wk, Wv, Wo, seg_len):
        B, S, Dm = x.shape
        H, Dh = (Wq.shape[1], Wq.shape[2])
        M = mem0.shape[1]
        scale = Dh ** (-0.5)
        n_seg = S // seg_len
        L = M + seg_len
        idx = jnp.arange(L)
        mask = (idx[:, None] < M) | (idx[:, None] >= idx[None, :])
        mem = mem0
        outs = []
        for s in range(n_seg):
            xs = x[:, s * seg_len:(s + 1) * seg_len, :].copy()
            h = jnp.concatenate([mem, xs], axis=1)
            q = jnp.einsum('btd,dhe->bhte', h, Wq)
            k = jnp.einsum('btd,dhe->bhte', h, Wk)
            v = jnp.einsum('btd,dhe->bhte', h, Wv)
            scores = jnp.einsum('bhqe,bhke->bhqk', q, k) * scale
            scores = jnp.where(mask[None, None], scores, -1000000000.0)
            p = _softmax(scores, axis=-1)
            o = jnp.einsum('bhqk,bhke->bhqe', p, v)
            o = jnp.einsum('bhte,hed->btd', o, Wo)
            mem = o[:, :M, :].copy()
            outs.append(o[:, M:, :])
        return jnp.concatenate(outs, axis=1)

    def _B_ref(x, w1, w2, w3, w4):
        B, S, D = x.shape
        h = _gelu(_layernorm(x, axis=-1) @ w1)
        c = D // 4
        g0 = jnp.pad(h[:, :, 0 * c:1 * c], ((0, 0), (1, 0), (0, 0)))[:, :S, :]
        g1 = jnp.pad(h[:, :, 1 * c:2 * c], ((0, 0), (0, 1), (0, 0)))[:, 1:, :]
        g2 = jnp.pad(h[:, :, 2 * c:3 * c], ((0, 0), (2, 0), (0, 0)))[:, :S, :]
        g3 = jnp.pad(h[:, :, 3 * c:], ((0, 0), (0, 2), (0, 0)))[:, 2:, :]
        hs = jnp.concatenate([g0, g1, g2, g3], axis=-1) @ w2
        x1 = x + hs
        h2 = _gelu(_layernorm(x1, axis=-1) @ w3) @ w4
        return x1 + h2
    x = A_x
    xn = _layernorm(x, axis=-1)
    s = _A_ref(xn, A_mem0, A_Wq, A_Wk, A_Wv, A_Wo, A_seg_len)
    g = _silu(_B_ref(xn, B_w1, B_w2, B_w3, B_w4))
    return x + s * g
```

```python
import functools

import jax
import jax.numpy as jnp
import numpy as np
from jax import lax
import jax.experimental.pallas as pl
import jax.experimental.pallas.tpu as pltpu

F32 = jnp.float32
BF16 = jnp.bfloat16
U32 = jnp.uint32

EPS = 1e-5
CH = 256
HALO = 8


def _layernorm(x):
    m = jnp.mean(x, axis=-1, keepdims=True)
    d = x - m
    v = jnp.mean(d * d, axis=-1, keepdims=True)
    return d * lax.rsqrt(v + EPS)


def _gelu(x):
    return jax.nn.gelu(x, approximate=True)


def _dot(a, b):
    return jnp.dot(a, b, preferred_element_type=F32)


def _kernel(
    x_hbm, mem0_ref, wq_hbm, wk_hbm, wv_hbm, wo_hbm, w1_hbm, w2_hbm, w3_hbm, w4_hbm,
    out_hbm,
    x_v, xn_v, h_v, g_v, w1_v, w2_v, w3_v, w4_v,
    stq_v, stk_v, stv_v, sto_v, wqkv_v, wo_v,
    x_sem, w_sem, st_sem, o_sem,
    *, S, D, H, Dh, M, SEG,
):
    n_ch = S // CH
    n_pair = H // 2
    d_ch = D // n_ch
    o_ch = (H * Dh) // n_ch
    c4 = D // 4

    def x_copy(c):
        r = pl.ds(c * CH, CH)
        return pltpu.make_async_copy(x_hbm.at[r], x_v.at[r], x_sem.at[c])

    w_copies = [
        pltpu.make_async_copy(src, dst, w_sem.at[i])
        for i, (src, dst) in enumerate(
            ((w1_hbm, w1_v), (w2_hbm, w2_v), (w3_hbm, w3_v), (w4_hbm, w4_v)))
    ]

    def stage_copies(c, slot):
        rq = pl.ds(pl.multiple_of(c * (d_ch * H), d_ch * H), d_ch * H)
        ro = pl.ds(pl.multiple_of(c * o_ch, o_ch), o_ch)
        return [
            pltpu.make_async_copy(wq_hbm.at[rq], stq_v.at[slot], st_sem.at[slot * 4 + 0]),
            pltpu.make_async_copy(wk_hbm.at[rq], stk_v.at[slot], st_sem.at[slot * 4 + 1]),
            pltpu.make_async_copy(wv_hbm.at[rq], stv_v.at[slot], st_sem.at[slot * 4 + 2]),
            pltpu.make_async_copy(wo_hbm.at[ro], sto_v.at[slot], st_sem.at[slot * 4 + 3]),
        ]

    x_copy(0).start()
    w_copies[0].start()
    for c in range(1, n_ch):
        x_copy(c).start()
    for cp in w_copies[1:]:
        cp.start()
    for cp in stage_copies(0, 0):
        cp.start()

    h_v[pl.ds(0, HALO), :] = jnp.zeros((HALO, D), F32)
    h_v[pl.ds(HALO + S, HALO), :] = jnp.zeros((HALO, D), F32)
    w_copies[0].wait()

    def phase0(c, carry):
        r0 = pl.multiple_of(c * CH, CH)
        rows = pl.ds(r0, CH)
        pltpu.make_async_copy(x_hbm.at[rows], x_v.at[rows], x_sem.at[c]).wait()
        xn = _layernorm(x_v[rows, :].astype(F32)).astype(BF16)
        xn_v[rows, :] = xn
        xn2 = _layernorm(xn.astype(F32)).astype(BF16)
        h_v[pl.ds(pl.multiple_of(r0 + HALO, HALO), CH), :] = _gelu(_dot(xn2, w1_v[...]))
        return carry

    lax.fori_loop(0, n_ch, phase0, 0)

    for cp in w_copies[1:]:
        cp.wait()

    def repack(c, slot):
        drow = pl.ds(pl.multiple_of(c * (d_ch // 2), d_ch // 2), d_ch // 2)
        for w, st in enumerate((stq_v, stk_v, stv_v)):
            st32 = st.at[slot].bitcast(U32)
            for p in range(n_pair):
                a = st32[pl.ds(p, d_ch // 2, stride=2 * n_pair), :]
                b = st32[pl.ds(n_pair + p, d_ch // 2, stride=2 * n_pair), :]
                lo = (a & jnp.uint32(0xFFFF)) | (b << 16)
                hi = (a >> 16) | (b & jnp.uint32(0xFFFF0000))
                wqkv_v[p, drow, pl.ds(2 * Dh * w, Dh)] = lo
                wqkv_v[p, drow, pl.ds(2 * Dh * w + Dh, Dh)] = hi
        orow = pl.ds(pl.multiple_of(c * (o_ch // 2), o_ch // 2), o_ch // 2)
        wo_v[orow, :] = pltpu.bitcast(sto_v[slot], U32)

    def phase1(c, carry):
        slot = c % 2
        for cp in stage_copies(c, slot):
            cp.wait()

        @pl.when(c + 1 < n_ch)
        def _():
            for cp in stage_copies(c + 1, 1 - slot):
                cp.start()

        r0 = pl.multiple_of(c * CH, CH)
        rows = pl.ds(r0, CH)
        win = pl.ds(r0, CH + 2 * HALO)
        parts = []
        for j, sh in enumerate((-1, 1, -2, 2)):
            hw = h_v[win, pl.ds(j * c4, c4)]
            parts.append(hw[HALO + sh:HALO + sh + CH].astype(BF16))
        hs = _dot(jnp.concatenate(parts, axis=1), w2_v[...])
        x1 = xn_v[rows, :].astype(F32) + hs
        u = _gelu(_dot(_layernorm(x1).astype(BF16), w3_v[...])).astype(BF16)
        y = x1 + _dot(u, w4_v[...])
        g_v[rows, :] = (y * jax.nn.sigmoid(y)).astype(g_v.dtype)
        repack(c, slot)
        return carry

    lax.fori_loop(0, n_ch, phase1, 0)

    L = M + SEG
    scale = Dh ** (-0.5)
    ri = lax.broadcasted_iota(jnp.int32, (2 * L, 2 * L), 0)
    ci = lax.broadcasted_iota(jnp.int32, (2 * L, 2 * L), 1)
    same_head = (ri >= L) == (ci >= L)
    rl = jnp.where(ri >= L, ri - L, ri)
    cl = jnp.where(ci >= L, ci - L, ci)
    visible = same_head & ((rl < M) | (rl >= cl))
    fill = jnp.where(same_head, F32(-1e9), F32(-jnp.inf))

    def heads_to_rows(y):
        return jnp.concatenate([y[:, :Dh], y[:, Dh:]], axis=0).astype(BF16)

    def attend(y):
        q = heads_to_rows(y[:, 0:2 * Dh])
        k = heads_to_rows(y[:, 2 * Dh:4 * Dh])
        v = heads_to_rows(y[:, 4 * Dh:6 * Dh])
        s = lax.dot_general(q, k, (((1,), (1,)), ((), ())), preferred_element_type=F32)
        s = jnp.where(visible, s * scale, fill)
        e = jnp.exp(s - jnp.max(s, axis=-1, keepdims=True))
        l = jnp.sum(e, axis=-1, keepdims=True)
        o = _dot(e.astype(BF16), v) / l
        return jnp.concatenate([o[:L], o[L:]], axis=1)

    def wqkv(p):
        return pltpu.bitcast(wqkv_v[p], BF16)

    def wo(p):
        return pltpu.bitcast(wo_v[pl.ds(p * Dh, Dh), :], BF16)

    def two_segments(j, mem):
        r0 = pl.multiple_of(j * (2 * SEG), 2 * SEG)
        rows = pl.ds(r0, 2 * SEG)
        xn = xn_v[rows, :].astype(F32)
        cut = SEG - M
        ha = jnp.concatenate([mem, xn[:SEG + M]], axis=0).astype(BF16)
        stash_y, stash_o = [], []
        acc_a = None
        for p in range(n_pair):
            y = _dot(ha, wqkv(p))
            stash_y.append(y[L:])
            o = attend(y[:L])
            stash_o.append(o[M + cut:])
            part = _dot(o[:M + cut].astype(BF16), wo(p))
            acc_a = part if acc_a is None else acc_a + part
        hb = jnp.concatenate([acc_a[:M], xn[SEG + M:]], axis=0).astype(BF16)
        acc_b = None
        for p in range(n_pair):
            y = _dot(hb, wqkv(p))
            o = attend(jnp.concatenate([y[:M], stash_y[p], y[M:]], axis=0))
            part = _dot(jnp.concatenate([o, stash_o[p]], axis=0).astype(BF16), wo(p))
            acc_b = part if acc_b is None else acc_b + part
        s = jnp.concatenate([acc_a[M:], acc_b[L:], acc_b[M:L]], axis=0)
        res = x_v[rows, :].astype(F32) + s * g_v[rows, :].astype(F32)
        x_v[rows, :] = res.astype(x_v.dtype)
        pltpu.make_async_copy(x_v.at[rows], out_hbm.at[rows], o_sem.at[0]).start()
        return acc_b[:M]

    lax.fori_loop(0, S // (2 * SEG), two_segments, mem0_ref[...].astype(F32))
    pltpu.make_async_copy(x_v, out_hbm, o_sem.at[0]).wait()


@functools.partial(jax.jit, static_argnames=("A_seg_len",))
def pallas_recurrent_scan__memory_aug_recurrent_mem_tr__mixer_s_mlp__prompt_kernel(
    A_x: jax.Array,
    A_mem0: jax.Array,
    A_Wq: jax.Array,
    A_Wk: jax.Array,
    A_Wv: jax.Array,
    A_Wo: jax.Array,
    A_seg_len: int,
    B_x: jax.Array,
    B_w1: jax.Array,
    B_w2: jax.Array,
    B_w3: jax.Array,
    B_w4: jax.Array,
):
    del B_x
    B, S, D = A_x.shape
    _, H, Dh = A_Wq.shape
    M = A_mem0.shape[1]
    F = B_w3.shape[1]
    SEG = int(A_seg_len)
    assert B == 1 and S % CH == 0 and S % (2 * SEG) == 0 and H % 2 == 0
    n_ch = S // CH
    d_ch = D // n_ch
    o_ch = (H * Dh) // n_ch

    any_spec = pl.BlockSpec(memory_space=pl.ANY)
    out = pl.pallas_call(
        functools.partial(_kernel, S=S, D=D, H=H, Dh=Dh, M=M, SEG=SEG),
        out_shape=jax.ShapeDtypeStruct((S, D), A_x.dtype),
        in_specs=[any_spec, pl.BlockSpec(memory_space=pltpu.VMEM)] + [any_spec] * 8,
        out_specs=any_spec,
        scratch_shapes=[
            pltpu.VMEM((S, D), BF16),
            pltpu.VMEM((S, D), BF16),
            pltpu.VMEM((S + 2 * HALO, D), F32),
            pltpu.VMEM((S, D), BF16),
            pltpu.VMEM((D, D), BF16),
            pltpu.VMEM((D, D), BF16),
            pltpu.VMEM((D, F), BF16),
            pltpu.VMEM((F, D), BF16),
            pltpu.VMEM((2, d_ch * H, Dh), BF16),
            pltpu.VMEM((2, d_ch * H, Dh), BF16),
            pltpu.VMEM((2, d_ch * H, Dh), BF16),
            pltpu.VMEM((2, o_ch, D), BF16),
            pltpu.VMEM((H // 2, D // 2, 6 * Dh), U32),
            pltpu.VMEM((H * Dh // 2, D), U32),
            pltpu.SemaphoreType.DMA((n_ch,)),
            pltpu.SemaphoreType.DMA((4,)),
            pltpu.SemaphoreType.DMA((8,)),
            pltpu.SemaphoreType.DMA((1,)),
        ],
        compiler_params=pltpu.CompilerParams(vmem_limit_bytes=120 * 1024 * 1024),
    )(
        A_x.reshape(S, D),
        A_mem0.reshape(M, D),
        A_Wq.reshape(D * H, Dh),
        A_Wk.reshape(D * H, Dh),
        A_Wv.reshape(D * H, Dh),
        A_Wo.reshape(H * Dh, D),
        B_w1, B_w2, B_w3, B_w4,
    )
    return out.reshape(B, S, D)
```

```python
import functools

import jax
import jax.numpy as jnp
import numpy as np
from jax import lax
import jax.experimental.pallas as pl
import jax.experimental.pallas.tpu as pltpu

F32 = jnp.float32
BF16 = jnp.bfloat16
U32 = jnp.uint32

EPS = 1e-5
CH = 256
G = 1
HALO = 8


def _layernorm(x):
    m = jnp.mean(x, axis=-1, keepdims=True)
    d = x - m
    v = jnp.mean(d * d, axis=-1, keepdims=True)
    return d * lax.rsqrt(v + EPS)


def _gelu(x):
    return jax.nn.gelu(x, approximate=True)


def _dot(a, b):
    return jnp.dot(a, b, preferred_element_type=F32)


def _kernel(
    x_hbm, mem0_ref, wq_hbm, wk_hbm, wv_hbm, wo_hbm, w1_hbm, w2_hbm, w3_hbm, w4_hbm,
    out_hbm,
    x_v, xn_v, h_v, g_v, w1_v, w2_v, w3_v, w4_v,
    stq_v, stk_v, stv_v, sto_v, wqkv_v, wo_v,
    x_sem, w_sem, st_sem, o_sem,
    *, S, D, H, Dh, M, SEG,
):
    n_ch = S // CH
    n_pair = H // 2
    d_ch = D // n_ch
    o_ch = (H * Dh) // n_ch
    c4 = D // 4

    def x_copy(c):
        r = pl.ds(c * CH, CH)
        return pltpu.make_async_copy(x_hbm.at[r], x_v.at[r], x_sem.at[c])

    w_copies = [
        pltpu.make_async_copy(src, dst, w_sem.at[i])
        for i, (src, dst) in enumerate(
            ((w1_hbm, w1_v), (w2_hbm, w2_v), (w3_hbm, w3_v), (w4_hbm, w4_v)))
    ]

    def stage_copies(c, slot):
        rq = pl.ds(pl.multiple_of(c * (d_ch * H), d_ch * H), d_ch * H)
        ro = pl.ds(pl.multiple_of(c * o_ch, o_ch), o_ch)
        return [
            pltpu.make_async_copy(wq_hbm.at[rq], stq_v.at[slot], st_sem.at[slot * 4 + 0]),
            pltpu.make_async_copy(wk_hbm.at[rq], stk_v.at[slot], st_sem.at[slot * 4 + 1]),
            pltpu.make_async_copy(wv_hbm.at[rq], stv_v.at[slot], st_sem.at[slot * 4 + 2]),
            pltpu.make_async_copy(wo_hbm.at[ro], sto_v.at[slot], st_sem.at[slot * 4 + 3]),
        ]

    x_copy(0).start()
    w_copies[0].start()

    h_v[pl.ds(0, HALO), :] = jnp.zeros((HALO, D), F32)
    h_v[pl.ds(HALO + S, HALO), :] = jnp.zeros((HALO, D), F32)
    w_copies[0].wait()
    for c in range(1, n_ch):
        x_copy(c).start()
    for cp in w_copies[1:]:
        cp.start()
    for cp in stage_copies(0, 0):
        cp.start()

    def phase0(c, carry):
        r0 = pl.multiple_of(c * CH, CH)
        rows = pl.ds(r0, CH)
        pltpu.make_async_copy(x_hbm.at[rows], x_v.at[rows], x_sem.at[c]).wait()
        xn = _layernorm(x_v[rows, :].astype(F32)).astype(BF16)
        xn_v[rows, :] = xn
        xn2 = _layernorm(xn.astype(F32)).astype(BF16)
        h_v[pl.ds(pl.multiple_of(r0 + HALO, HALO), CH), :] = _gelu(_dot(xn2, w1_v[...]))
        return carry

    lax.fori_loop(0, n_ch, phase0, 0)

    for cp in w_copies[1:]:
        cp.wait()

    def repack(c, slot):
        drow = pl.ds(pl.multiple_of(c * (d_ch // 2), d_ch // 2), d_ch // 2)
        for w, st in enumerate((stq_v, stk_v, stv_v)):
            st32 = st.at[slot].bitcast(U32)
            for p in range(n_pair):
                a = st32[pl.ds(p, d_ch // 2, stride=2 * n_pair), :]
                b = st32[pl.ds(n_pair + p, d_ch // 2, stride=2 * n_pair), :]
                lo = (a & jnp.uint32(0xFFFF)) | (b << 16)
                hi = (a >> 16) | (b & jnp.uint32(0xFFFF0000))
                wqkv_v[p, drow, pl.ds(2 * Dh * w, Dh)] = lo
                wqkv_v[p, drow, pl.ds(2 * Dh * w + Dh, Dh)] = hi
        orow = pl.ds(pl.multiple_of(c * (o_ch // 2), o_ch // 2), o_ch // 2)
        wo_v[orow, :] = pltpu.bitcast(sto_v[slot], U32)

    def phase1(c, carry):
        slot = c % 2
        for cp in stage_copies(c, slot):
            cp.wait()

        @pl.when(c + 1 < n_ch)
        def _():
            for cp in stage_copies(c + 1, 1 - slot):
                cp.start()

        r0 = pl.multiple_of(c * CH, CH)
        rows = pl.ds(r0, CH)
        win = pl.ds(r0, CH + 2 * HALO)
        parts = []
        for j, sh in enumerate((-1, 1, -2, 2)):
            hw = h_v[win, pl.ds(j * c4, c4)]
            parts.append(hw[HALO + sh:HALO + sh + CH].astype(BF16))
        hs = _dot(jnp.concatenate(parts, axis=1), w2_v[...])
        x1 = xn_v[rows, :].astype(F32) + hs
        u = _gelu(_dot(_layernorm(x1).astype(BF16), w3_v[...])).astype(BF16)
        y = x1 + _dot(u, w4_v[...])
        g_v[rows, :] = (y * jax.nn.sigmoid(y)).astype(g_v.dtype)
        repack(c, slot)
        return carry

    lax.fori_loop(0, n_ch, phase1, 0)

    L = M + SEG
    scale = Dh ** (-0.5)
    ri = lax.broadcasted_iota(jnp.int32, (2 * L, 2 * L), 0)
    ci = lax.broadcasted_iota(jnp.int32, (2 * L, 2 * L), 1)
    same_head = (ri >= L) == (ci >= L)
    rl = jnp.where(ri >= L, ri - L, ri)
    cl = jnp.where(ci >= L, ci - L, ci)
    visible = same_head & ((rl < M) | (rl >= cl))
    fill = jnp.where(same_head, F32(-1e9), F32(-jnp.inf))

    def heads_to_rows(y):
        return jnp.concatenate([y[:, :Dh], y[:, Dh:]], axis=0).astype(BF16)

    def wqkv(p):
        return pltpu.bitcast(wqkv_v[p], BF16)

    def wo(p, n):
        return pltpu.bitcast(wo_v[pl.ds(p * Dh, n * Dh), :], BF16)

    def segment(h, get_y, get_o):
        n_grp = n_pair // G
        qkv, ev, outs = {}, {}, {}
        acc = None
        for t in range(n_grp + 3):
            if t < n_grp:
                for p in range(t * G, (t + 1) * G):
                    y = get_y(p, _dot(h, wqkv(p)))
                    qkv[p] = [heads_to_rows(y[:, 2 * Dh * i:2 * Dh * (i + 1)]) for i in range(3)]
            if 0 <= t - 1 < n_grp:
                for p in range((t - 1) * G, t * G):
                    q, k, v = qkv.pop(p)
                    s = lax.dot_general(q, k, (((1,), (1,)), ((), ())), preferred_element_type=F32)
                    s = jnp.where(visible, s * scale, fill)
                    e = jnp.exp(s - jnp.max(s, axis=-1, keepdims=True))
                    l = jnp.sum(e, axis=-1, keepdims=True)
                    r = pl.reciprocal(l, approx=True)
                    ev[p] = (e.astype(BF16), v, r * (2.0 - l * r))
            if 0 <= t - 2 < n_grp:
                for p in range((t - 2) * G, (t - 1) * G):
                    e, v, r = ev.pop(p)
                    o = _dot(e, v) * r
                    o = jnp.concatenate([o[:L], o[L:]], axis=1)
                    outs[p] = get_o(p, o).astype(BF16)
            if 0 <= t - 3 < n_grp:
                p0 = (t - 3) * G
                o = jnp.concatenate([outs.pop(p) for p in range(p0, p0 + G)], axis=1)
                part = _dot(o, wo(p0, G))
                acc = part if acc is None else acc + part
        return acc

    def two_segments(j, mem):
        r0 = pl.multiple_of(j * (2 * SEG), 2 * SEG)
        rows = pl.ds(r0, 2 * SEG)
        xn = xn_v[rows, :].astype(F32)
        stash_y, stash_o = {}, {}

        def y_a(p, y):
            stash_y[p] = y[L:]
            return y[:L]

        def o_a(p, o):
            stash_o[p] = o[SEG:]
            return o[:SEG]

        acc_a = segment(jnp.concatenate([mem, xn[:L]], axis=0).astype(BF16), y_a, o_a)

        def y_b(p, y):
            return jnp.concatenate([y[:M], stash_y[p], y[M:]], axis=0)

        def o_b(p, o):
            return jnp.concatenate([o, stash_o[p]], axis=0)

        acc_b = segment(jnp.concatenate([acc_a[:M], xn[L:]], axis=0).astype(BF16), y_b, o_b)

        s = jnp.concatenate([acc_a[M:], acc_b[L:], acc_b[M:L]], axis=0)
        res = x_v[rows, :].astype(F32) + s * g_v[rows, :].astype(F32)
        x_v[rows, :] = res.astype(x_v.dtype)
        pltpu.make_async_copy(x_v.at[rows], out_hbm.at[rows], o_sem.at[0]).start()
        return acc_b[:M]

    lax.fori_loop(0, S // (2 * SEG), two_segments, mem0_ref[...].astype(F32))
    pltpu.make_async_copy(x_v, out_hbm, o_sem.at[0]).wait()


@functools.partial(jax.jit, static_argnames=("A_seg_len",))
def pallas_recurrent_scan__memory_aug_recurrent_mem_tr__mixer_s_mlp__prompt_kernel(
    A_x: jax.Array,
    A_mem0: jax.Array,
    A_Wq: jax.Array,
    A_Wk: jax.Array,
    A_Wv: jax.Array,
    A_Wo: jax.Array,
    A_seg_len: int,
    B_x: jax.Array,
    B_w1: jax.Array,
    B_w2: jax.Array,
    B_w3: jax.Array,
    B_w4: jax.Array,
):
    del B_x
    B, S, D = A_x.shape
    _, H, Dh = A_Wq.shape
    M = A_mem0.shape[1]
    F = B_w3.shape[1]
    SEG = int(A_seg_len)
    assert B == 1 and S % CH == 0 and S % (2 * SEG) == 0 and H % 2 == 0
    n_ch = S // CH
    d_ch = D // n_ch
    o_ch = (H * Dh) // n_ch

    any_spec = pl.BlockSpec(memory_space=pl.ANY)
    out = pl.pallas_call(
        functools.partial(_kernel, S=S, D=D, H=H, Dh=Dh, M=M, SEG=SEG),
        out_shape=jax.ShapeDtypeStruct((S, D), A_x.dtype),
        in_specs=[any_spec, pl.BlockSpec(memory_space=pltpu.VMEM)] + [any_spec] * 8,
        out_specs=any_spec,
        scratch_shapes=[
            pltpu.VMEM((S, D), BF16),
            pltpu.VMEM((S, D), BF16),
            pltpu.VMEM((S + 2 * HALO, D), F32),
            pltpu.VMEM((S, D), BF16),
            pltpu.VMEM((D, D), BF16),
            pltpu.VMEM((D, D), BF16),
            pltpu.VMEM((D, F), BF16),
            pltpu.VMEM((F, D), BF16),
            pltpu.VMEM((2, d_ch * H, Dh), BF16),
            pltpu.VMEM((2, d_ch * H, Dh), BF16),
            pltpu.VMEM((2, d_ch * H, Dh), BF16),
            pltpu.VMEM((2, o_ch, D), BF16),
            pltpu.VMEM((H // 2, D // 2, 6 * Dh), U32),
            pltpu.VMEM((H * Dh // 2, D), U32),
            pltpu.SemaphoreType.DMA((n_ch,)),
            pltpu.SemaphoreType.DMA((4,)),
            pltpu.SemaphoreType.DMA((8,)),
            pltpu.SemaphoreType.DMA((1,)),
        ],
        compiler_params=pltpu.CompilerParams(vmem_limit_bytes=120 * 1024 * 1024),
    )(
        A_x.reshape(S, D),
        A_mem0.reshape(M, D),
        A_Wq.reshape(D * H, Dh),
        A_Wk.reshape(D * H, Dh),
        A_Wv.reshape(D * H, Dh),
        A_Wo.reshape(H * Dh, D),
        B_w1, B_w2, B_w3, B_w4,
    )
    return out.reshape(B, S, D)
```

```python
import functools

import jax
import jax.numpy as jnp
import numpy as np
from jax import lax
import jax.experimental.pallas as pl
import jax.experimental.pallas.tpu as pltpu

F32 = jnp.float32
BF16 = jnp.bfloat16
U32 = jnp.uint32

EPS = 1e-5
CH = 256
FC = 512
RO = 64
G = 2
HALO = 8


def _layernorm(x):
    m = jnp.mean(x, axis=-1, keepdims=True)
    d = x - m
    v = jnp.mean(d * d, axis=-1, keepdims=True)
    return d * lax.rsqrt(v + EPS)


def _gelu(x):
    return jax.nn.gelu(x, approximate=True)


def _dot(a, b):
    return jnp.dot(a, b, preferred_element_type=F32)


def _kernel(
    x_hbm, mem0_ref, wq_hbm, wk_hbm, wv_hbm, wo_hbm, w1_hbm, w2_hbm, w3_hbm, w4_hbm,
    out_hbm,
    x_v, xn_v, n_v, n3_v, h_v, g_v, w1_v, w2_v, w3_v, w4_v,
    stq_v, stk_v, stv_v, sto_v, wqkv_v, wo_v,
    x_sem, w_sem, st_sem, o_sem,
    *, S, D, F, H, Dh, M, SEG,
):
    n_ch = S // CH
    n_pair = H // 2
    d_ch = D // n_ch
    o_ch = (H * Dh) // n_ch
    c4 = D // 4

    def x_copy(c):
        r = pl.ds(c * CH, CH)
        return pltpu.make_async_copy(x_hbm.at[r], x_v.at[r], x_sem.at[c])

    w_copies = [
        pltpu.make_async_copy(src, dst, w_sem.at[i])
        for i, (src, dst) in enumerate(
            ((w1_hbm, w1_v), (w2_hbm, w2_v), (w3_hbm, w3_v), (w4_hbm, w4_v)))
    ]

    def stage_copies(c, slot):
        rq = pl.ds(pl.multiple_of(c * (d_ch * H), d_ch * H), d_ch * H)
        ro = pl.ds(pl.multiple_of(c * o_ch, o_ch), o_ch)
        return [
            pltpu.make_async_copy(wq_hbm.at[rq], stq_v.at[slot], st_sem.at[slot * 4 + 0]),
            pltpu.make_async_copy(wk_hbm.at[rq], stk_v.at[slot], st_sem.at[slot * 4 + 1]),
            pltpu.make_async_copy(wv_hbm.at[rq], stv_v.at[slot], st_sem.at[slot * 4 + 2]),
            pltpu.make_async_copy(wo_hbm.at[ro], sto_v.at[slot], st_sem.at[slot * 4 + 3]),
        ]

    x_copy(0).start()
    w_copies[0].start()

    def chunk(c):
        return pl.ds(pl.multiple_of(c * CH, CH), CH)

    def with_side_jobs(y, jobs):
        if not jobs:
            return y
        n_t = y.shape[1] // 128
        per = -(-len(jobs) // n_t)
        step = y.shape[0] // per
        cols = []
        for j in range(n_t):
            col = y[:, 128 * j:128 * (j + 1)]
            mine = jobs[j * len(jobs) // n_t:(j + 1) * len(jobs) // n_t]
            rows = []
            for i, job in enumerate(mine):
                rows += [col[i * step:i * step + 8] + job(), col[i * step + 8:(i + 1) * step]]
            rows.append(col[len(mine) * step:])
            cols.append(jnp.concatenate([r for r in rows if r.shape[0]], axis=0))
        return jnp.concatenate(cols, axis=1)

    n_v[pl.ds(S, 16 * n_ch), :] = jnp.zeros((16 * n_ch, D), BF16)
    wqkv_v[n_pair, pl.ds(0, 8 * n_ch), pl.ds(0, Dh)] = jnp.zeros((8 * n_ch, Dh), U32)
    wo_v[pl.ds(H * Dh // 2, 8 * n_ch), :] = jnp.zeros((8 * n_ch, D), U32)

    h_v[pl.ds(HALO, 8), :] = jnp.zeros((8, D), F32)
    h_v[pl.ds(HALO + S - 8, 8), :] = jnp.zeros((8, D), F32)

    def norm_jobs(c):
        def job(i):
            r = pl.ds(pl.multiple_of(c * CH + i * 16, 16), 16)
            xn = _layernorm(x_v[r, :].astype(F32)).astype(BF16)
            xn_v[r, :] = xn
            n_v[r, :] = _layernorm(xn.astype(F32)).astype(BF16)
            z = n_v[pl.ds(pl.multiple_of(S + c * 16, 16), 16), pl.ds(0, 128)]
            return z.astype(F32)[:8]
        return [functools.partial(job, i) for i in range(CH // 16)]

    def w1_stage(c, jobs=()):
        h = _gelu(with_side_jobs(_dot(n_v[chunk(c), :], w1_v[...]), jobs))
        win = h_v.at[pl.ds(pl.multiple_of(c * CH, CH), CH + 2 * HALO)]
        for j, sh in enumerate((-1, 1, -2, 2)):
            win[pl.ds(HALO - sh, CH), pl.ds(j * c4, c4)] = h[:, j * c4:(j + 1) * c4]

    def w2_stage(c, jobs=()):
        hs = h_v[pl.ds(pl.multiple_of(c * CH + HALO, HALO), CH), :].astype(BF16)
        x1 = xn_v[chunk(c), :].astype(F32) + with_side_jobs(_dot(hs, w2_v[...]), jobs)
        g_v[chunk(c), :] = x1
        n3_v[chunk(c), :] = _layernorm(x1).astype(BF16)

    x_copy(0).wait()
    for job in norm_jobs(0):
        job()
    w_copies[0].wait()
    for c in range(1, n_ch):
        x_copy(c).start()
    w_copies[1].start()

    for c in range(2):
        x_copy(c + 1).wait()
        w1_stage(c, norm_jobs(c + 1))
    for cp in w_copies[2:] + stage_copies(0, 0) + stage_copies(1, 1):
        cp.start()
    w_copies[1].wait()
    for c in range(3, n_ch):
        x_copy(c).wait()

    def phase0(c, carry):
        jobs = norm_jobs(c + 1)
        w2_stage(c - 2, jobs[:len(jobs) // 2])
        w1_stage(c, jobs[len(jobs) // 2:])
        return carry

    lax.fori_loop(2, n_ch - 1, phase0, 0)
    w2_stage(n_ch - 3)
    w1_stage(n_ch - 1)
    w2_stage(n_ch - 2)
    w2_stage(n_ch - 1)

    for cp in w_copies[2:]:
        cp.wait()

    sub = lax.broadcasted_iota(jnp.int32, (8, Dh), 0)

    def transpose8(vs):
        for s in (4, 2, 1):
            upper = (sub & s) != 0
            out = list(vs)
            for i in range(8):
                if not i & s:
                    a, b = vs[i], vs[i + s]
                    out[i] = jnp.where(upper, pltpu.roll(b, s, 0), a)
                    out[i + s] = jnp.where(upper, b, pltpu.roll(a, 8 - s, 0))
            vs = out
        return vs

    def repack_qkv(c, slot, w, blk, grp):
        st = (stq_v, stk_v, stv_v)[w]
        src = [pltpu.bitcast(st[slot, pl.ds((blk * 16 + d) * H + grp * 16, 16), :], U32)
               for d in range(16)]
        drow = pl.ds(pl.multiple_of(c * (d_ch // 2) + blk * 8, 8), 8)
        for j in range(2):
            words = [
                pltpu.pack_elementwise([src[2 * i] >> 16, src[2 * i + 1] >> 16] if j
                                       else [src[2 * i], src[2 * i + 1]],
                                       packed_dtype=jnp.uint16)
                for i in range(8)]
            for p, tile in enumerate(transpose8(words)):
                wqkv_v[grp * 8 + p, drow, pl.ds((2 * w + j) * Dh, Dh)] = tile.astype(U32)
        z = wqkv_v[n_pair, pl.ds(pl.multiple_of(c * 8, 8), 8), pl.ds(0, Dh)]
        return pltpu.bitcast(z, F32)

    def repack_o(c, slot, i):
        orow = pl.ds(pl.multiple_of(c * (o_ch // 2) + i * (RO // 2), RO // 2), RO // 2)
        wo_v[orow, :] = pltpu.bitcast(sto_v[slot, pl.ds(i * RO, RO), :], U32)
        z = wo_v[pl.ds(pl.multiple_of(H * Dh // 2 + c * 8, 8), 8), pl.ds(0, 128)]
        return pltpu.bitcast(z, F32)

    def phase1(c, carry):
        slot = c % 2
        for cp in stage_copies(c, slot):
            cp.wait()

        n_f = F // FC
        jobs = [functools.partial(repack_qkv, c, slot, w, blk, grp)
                for w in range(3) for blk in range(d_ch // 16) for grp in range(H // 16)]
        jobs += [functools.partial(repack_o, c, slot, i) for i in range(o_ch // RO)]

        def share(k):
            return jobs[k * len(jobs) // (2 * n_f):(k + 1) * len(jobs) // (2 * n_f)]

        rows = chunk(c)
        u = {}
        for t in range(n_f + 1):
            if t < n_f:
                up = _dot(n3_v[rows, :], w3_v[:, pl.ds(t * FC, FC)])
                u[t] = _gelu(with_side_jobs(up, share(max(2 * t - 1, 0)))).astype(BF16)
            if t >= 1:
                down = _dot(u.pop(t - 1), w4_v[pl.ds((t - 1) * FC, FC), :])
                y = g_v[rows, :] + with_side_jobs(down, share(min(2 * t, 2 * n_f - 1)))
                if t == n_f:
                    y = y * jax.nn.sigmoid(y)
                g_v[rows, :] = y

        @pl.when(c + 2 < n_ch)
        def _():
            for cp in stage_copies(c + 2, slot):
                cp.start()

        return carry

    lax.fori_loop(0, n_ch, phase1, 0)

    L = M + SEG
    scale = Dh ** (-0.5)
    ri = lax.broadcasted_iota(jnp.int32, (2 * L, 2 * L), 0)
    ci = lax.broadcasted_iota(jnp.int32, (2 * L, 2 * L), 1)
    same_head = (ri >= L) == (ci >= L)
    rl = jnp.where(ri >= L, ri - L, ri)
    cl = jnp.where(ci >= L, ci - L, ci)
    visible = same_head & ((rl < M) | (rl >= cl))
    fill = jnp.where(same_head, F32(-1e9), F32(-jnp.inf))

    def heads_to_rows(y):
        return jnp.concatenate([y[:, :Dh], y[:, Dh:]], axis=0).astype(BF16)

    def wqkv(p):
        return pltpu.bitcast(wqkv_v[p], BF16)

    def wo(p, n):
        return pltpu.bitcast(wo_v[pl.ds(p * Dh, n * Dh), :], BF16)

    def segment(h, get_y, get_o):
        n_grp = n_pair // G
        qkv, ev, outs = {}, {}, {}
        acc = None
        for t in range(n_grp + 3):
            if t < n_grp:
                for p in range(t * G, (t + 1) * G):
                    y = get_y(p, _dot(h, wqkv(p)))
                    qkv[p] = [heads_to_rows(y[:, 2 * Dh * i:2 * Dh * (i + 1)]) for i in range(3)]
            if 0 <= t - 1 < n_grp:
                for p in range((t - 1) * G, t * G):
                    q, k, v = qkv.pop(p)
                    s = lax.dot_general(q, k, (((1,), (1,)), ((), ())), preferred_element_type=F32)
                    s = jnp.where(visible, s * scale, fill)
                    e = jnp.exp(s - jnp.max(s, axis=-1, keepdims=True))
                    l = jnp.sum(e, axis=-1, keepdims=True)
                    r = pl.reciprocal(l, approx=True)
                    ev[p] = (e.astype(BF16), v, r * (2.0 - l * r))
            if 0 <= t - 2 < n_grp:
                for p in range((t - 2) * G, (t - 1) * G):
                    e, v, r = ev.pop(p)
                    o = _dot(e, v) * r
                    o = jnp.concatenate([o[:L], o[L:]], axis=1)
                    outs[p] = get_o(p, o).astype(BF16)
            if 0 <= t - 3 < n_grp:
                p0 = (t - 3) * G
                o = jnp.concatenate([outs.pop(p) for p in range(p0, p0 + G)], axis=1)
                part = _dot(o, wo(p0, G))
                acc = part if acc is None else acc + part
        return acc

    def two_segments(j, mem):
        r0 = pl.multiple_of(j * (2 * SEG), 2 * SEG)
        rows = pl.ds(r0, 2 * SEG)
        xn = xn_v[rows, :].astype(F32)
        stash_y, stash_o = {}, {}

        def y_a(p, y):
            stash_y[p] = y[L:]
            return y[:L]

        def o_a(p, o):
            stash_o[p] = o[SEG:]
            return o[:SEG]

        acc_a = segment(jnp.concatenate([mem, xn[:L]], axis=0).astype(BF16), y_a, o_a)

        def y_b(p, y):
            return jnp.concatenate([y[:M], stash_y[p], y[M:]], axis=0)

        def o_b(p, o):
            return jnp.concatenate([o, stash_o[p]], axis=0)

        acc_b = segment(jnp.concatenate([acc_a[:M], xn[L:]], axis=0).astype(BF16), y_b, o_b)

        s = jnp.concatenate([acc_a[M:], acc_b[L:], acc_b[M:L]], axis=0)
        res = x_v[rows, :].astype(F32) + s * g_v[rows, :]
        x_v[rows, :] = res.astype(x_v.dtype)
        pltpu.make_async_copy(x_v.at[rows], out_hbm.at[rows], o_sem.at[0]).start()
        return acc_b[:M]

    lax.fori_loop(0, S // (2 * SEG), two_segments, mem0_ref[...].astype(F32))
    pltpu.make_async_copy(x_v, out_hbm, o_sem.at[0]).wait()


@functools.partial(jax.jit, static_argnames=("A_seg_len",))
def pallas_recurrent_scan__memory_aug_recurrent_mem_tr__mixer_s_mlp__prompt_kernel(
    A_x: jax.Array,
    A_mem0: jax.Array,
    A_Wq: jax.Array,
    A_Wk: jax.Array,
    A_Wv: jax.Array,
    A_Wo: jax.Array,
    A_seg_len: int,
    B_x: jax.Array,
    B_w1: jax.Array,
    B_w2: jax.Array,
    B_w3: jax.Array,
    B_w4: jax.Array,
):
    del B_x
    B, S, D = A_x.shape
    _, H, Dh = A_Wq.shape
    M = A_mem0.shape[1]
    F = B_w3.shape[1]
    SEG = int(A_seg_len)
    assert B == 1 and S % CH == 0 and S % (2 * SEG) == 0 and H % 2 == 0
    n_ch = S // CH
    d_ch = D // n_ch
    o_ch = (H * Dh) // n_ch

    any_spec = pl.BlockSpec(memory_space=pl.ANY)
    out = pl.pallas_call(
        functools.partial(_kernel, S=S, D=D, F=F, H=H, Dh=Dh, M=M, SEG=SEG),
        out_shape=jax.ShapeDtypeStruct((S, D), A_x.dtype),
        in_specs=[any_spec, pl.BlockSpec(memory_space=pltpu.VMEM)] + [any_spec] * 8,
        out_specs=any_spec,
        scratch_shapes=[
            pltpu.VMEM((S, D), BF16),
            pltpu.VMEM((S, D), BF16),
            pltpu.VMEM((S + 16 * n_ch, D), BF16),
            pltpu.VMEM((S, D), BF16),
            pltpu.VMEM((S + 2 * HALO, D), F32),
            pltpu.VMEM((S, D), F32),
            pltpu.VMEM((D, D), BF16),
            pltpu.VMEM((D, D), BF16),
            pltpu.VMEM((D, F), BF16),
            pltpu.VMEM((F, D), BF16),
            pltpu.VMEM((2, d_ch * H, Dh), BF16),
            pltpu.VMEM((2, d_ch * H, Dh), BF16),
            pltpu.VMEM((2, d_ch * H, Dh), BF16),
            pltpu.VMEM((2, o_ch, D), BF16),
            pltpu.VMEM((H // 2 + 1, D // 2, 6 * Dh), U32),
            pltpu.VMEM((H * Dh // 2 + 8 * n_ch, D), U32),
            pltpu.SemaphoreType.DMA((n_ch,)),
            pltpu.SemaphoreType.DMA((4,)),
            pltpu.SemaphoreType.DMA((8,)),
            pltpu.SemaphoreType.DMA((1,)),
        ],
        compiler_params=pltpu.CompilerParams(vmem_limit_bytes=120 * 1024 * 1024),
    )(
        A_x.reshape(S, D),
        A_mem0.reshape(M, D),
        A_Wq.reshape(D * H, Dh),
        A_Wk.reshape(D * H, Dh),
        A_Wv.reshape(D * H, Dh),
        A_Wo.reshape(H * Dh, D),
        B_w1, B_w2, B_w3, B_w4,
    )
    return out.reshape(B, S, D)
```

```python
import functools

import jax
import jax.numpy as jnp
import numpy as np
from jax import lax
import jax.experimental.pallas as pl
import jax.experimental.pallas.tpu as pltpu

F32 = jnp.float32
BF16 = jnp.bfloat16
U32 = jnp.uint32

EPS = 1e-5
CH = 256
FC = 512
RN = 16
RO = 64
G = 2
HALO = 8


def _layernorm(x):
    m = jnp.mean(x, axis=-1, keepdims=True)
    d = x - m
    v = jnp.mean(d * d, axis=-1, keepdims=True)
    return d * lax.rsqrt(v + EPS)


def _gelu(x):
    return jax.nn.gelu(x, approximate=True)


def _dot(a, b):
    return jnp.dot(a, b, preferred_element_type=F32)


def _kernel(
    x_hbm, mem0_ref, wq_hbm, wk_hbm, wv_hbm, wo_hbm, w1_hbm, w2_hbm, w3_hbm, w4_hbm,
    out_hbm,
    x_v, xn_v, n_v, n3_v, h_v, g_v, w1_v, w2_v, w3_v, w4_v,
    stq_v, stk_v, stv_v, sto_v, wqkv_v, wo_v,
    x_sem, w_sem, st_sem, o_sem,
    *, S, D, F, H, Dh, M, SEG,
):
    n_ch = S // CH
    n_pair = H // 2
    d_ch = D // n_ch
    o_ch = (H * Dh) // n_ch
    c4 = D // 4

    def x_copy(c):
        r = pl.ds(pl.multiple_of(c * CH, CH), CH)
        return pltpu.make_async_copy(x_hbm.at[r], x_v.at[r], x_sem.at[c])

    w_copies = [
        pltpu.make_async_copy(src, dst, w_sem.at[i])
        for i, (src, dst) in enumerate(
            ((w1_hbm, w1_v), (w2_hbm, w2_v), (w3_hbm, w3_v), (w4_hbm, w4_v)))
    ]

    def stage_copies(c, slot):
        rq = pl.ds(pl.multiple_of(c * (d_ch * H), d_ch * H), d_ch * H)
        ro = pl.ds(pl.multiple_of(c * o_ch, o_ch), o_ch)
        return [
            pltpu.make_async_copy(wq_hbm.at[rq], stq_v.at[slot], st_sem.at[slot * 4 + 0]),
            pltpu.make_async_copy(wk_hbm.at[rq], stk_v.at[slot], st_sem.at[slot * 4 + 1]),
            pltpu.make_async_copy(wv_hbm.at[rq], stv_v.at[slot], st_sem.at[slot * 4 + 2]),
            pltpu.make_async_copy(wo_hbm.at[ro], sto_v.at[slot], st_sem.at[slot * 4 + 3]),
        ]

    x_copy(0).start()
    w_copies[0].start()
    x_copy(1).start()

    def chunk(c):
        return pl.ds(pl.multiple_of(c * CH, CH), CH)

    def dot_with_jobs(a, w, jobs):
        if jobs:
            w = pltpu.bitcast(w, U32)
            n_t, half = w.shape[1] // 128, w.shape[0] // 2
            cols = []
            for j in range(n_t):
                rows = []
                for i in range(2):
                    part = w[i * half:(i + 1) * half, 128 * j:128 * (j + 1)]
                    k = 2 * j + i - 1
                    if k >= 0:
                        top = part[:8]
                        for job in jobs[k * len(jobs) // (2 * n_t - 1):
                                        (k + 1) * len(jobs) // (2 * n_t - 1)]:
                            top = top | job()
                        part = jnp.concatenate([top, part[8:]], axis=0)
                    rows.append(part)
                cols.append(jnp.concatenate(rows, axis=0))
            w = pltpu.bitcast(jnp.concatenate(cols, axis=1), BF16)
        return _dot(a, w)

    def with_side_jobs(y, jobs):
        if not jobs:
            return y
        n_t = y.shape[1] // 128
        per = -(-len(jobs) // n_t)
        step = y.shape[0] // per
        cols = []
        for j in range(n_t):
            col = y[:, 128 * j:128 * (j + 1)]
            mine = jobs[j * len(jobs) // n_t:(j + 1) * len(jobs) // n_t]
            rows = []
            for i, job in enumerate(mine):
                rows += [col[i * step:i * step + 8] + pltpu.bitcast(job(), F32), col[i * step + 8:(i + 1) * step]]
            rows.append(col[len(mine) * step:])
            cols.append(jnp.concatenate([r for r in rows if r.shape[0]], axis=0))
        return jnp.concatenate(cols, axis=1)

    n_v[pl.ds(S, 16 * n_ch), pl.ds(0, 128)] = jnp.zeros((16 * n_ch, 128), BF16)
    n3_v[pl.ds(S, 16 * n_ch), pl.ds(0, 128)] = jnp.zeros((16 * n_ch, 128), BF16)
    wqkv_v[n_pair, pl.ds(0, 8 * n_ch), pl.ds(0, Dh)] = jnp.zeros((8 * n_ch, Dh), U32)
    wo_v[pl.ds(H * Dh // 2, 8 * n_ch), pl.ds(0, 128)] = jnp.zeros((8 * n_ch, 128), U32)

    h_v[pl.ds(HALO, 8), :] = jnp.zeros((8, D), F32)
    h_v[pl.ds(HALO + S - 8, 8), :] = jnp.zeros((8, D), F32)

    def norm_jobs(c):
        def job(i):
            r = pl.ds(pl.multiple_of(c * CH + i * RN, RN), RN)
            xn = _layernorm(x_v[r, :].astype(F32)).astype(BF16)
            xn_v[r, :] = xn
            n_v[r, :] = _layernorm(xn.astype(F32)).astype(BF16)
            z = n_v[pl.ds(pl.multiple_of(S + c * 16, 16), 16), pl.ds(0, 128)]
            return pltpu.bitcast(z, U32)
        return [functools.partial(job, i) for i in range(CH // RN)]

    def w1_stage(c, jobs=()):
        h = _gelu(dot_with_jobs(n_v[chunk(c), :], w1_v[...], jobs))
        win = h_v.at[pl.ds(pl.multiple_of(c * CH, CH), CH + 2 * HALO)]
        for j, sh in enumerate((-1, 1, -2, 2)):
            win[pl.ds(HALO - sh, CH), pl.ds(j * c4, c4)] = h[:, j * c4:(j + 1) * c4]

    def w2_stage(c, jobs=()):
        hs = h_v[pl.ds(pl.multiple_of(c * CH + HALO, HALO), CH), :].astype(BF16)
        g_v[chunk(c), :] = xn_v[chunk(c), :].astype(F32) + dot_with_jobs(hs, w2_v[...], jobs)

    def norm3_jobs(c):
        def job(i):
            r = pl.ds(pl.multiple_of(c * CH + i * RN, RN), RN)
            n3_v[r, :] = _layernorm(g_v[r, :]).astype(BF16)
            z = n3_v[pl.ds(pl.multiple_of(S + c * 16, 16), 16), pl.ds(0, 128)]
            return pltpu.bitcast(z, U32)
        return [functools.partial(job, i) for i in range(CH // RN)]

    x_copy(0).wait()
    for job in norm_jobs(0):
        job()
    w_copies[0].wait()
    x_copy(2).start()
    w_copies[1].start()

    @pl.loop(0, n_ch + 2)
    def _(c):
        @pl.when(c == 1)
        def _():
            for i in range(3, n_ch):
                x_copy(i).start()

        @pl.when(c == 2)
        def _():
            w_copies[1].wait()
            for cp in w_copies[2:] + stage_copies(0, 0) + stage_copies(1, 1):
                cp.start()

        @pl.when(c + 1 < n_ch)
        def _():
            x_copy(c + 1).wait()

        jobs = norm_jobs(jnp.minimum(c + 1, n_ch - 1))
        half = len(jobs) // 2

        @pl.when(c < 2)
        def _():
            for job in jobs[:half]:
                job()

        @pl.when(c >= 2)
        def _():
            w2_stage(c - 2, jobs[:half])

        @pl.when(c < n_ch)
        def _():
            w1_stage(c, jobs[half:])

    for job in norm3_jobs(0):
        job()

    for cp in w_copies[2:]:
        cp.wait()

    sub = lax.broadcasted_iota(jnp.int32, (8, Dh), 0)

    def transpose8(vs):
        for s in (4, 2, 1):
            upper = (sub & s) != 0
            out = list(vs)
            for i in range(8):
                if not i & s:
                    a, b = vs[i], vs[i + s]
                    out[i] = jnp.where(upper, pltpu.roll(b, s, 0), a)
                    out[i + s] = jnp.where(upper, b, pltpu.roll(a, 8 - s, 0))
            vs = out
        return vs

    def repack_qkv(c, slot, w, blk, grp):
        st = (stq_v, stk_v, stv_v)[w]
        src = [pltpu.bitcast(st[slot, pl.ds((blk * 16 + d) * H + grp * 16, 16), :], U32)
               for d in range(16)]
        drow = pl.ds(pl.multiple_of(c * (d_ch // 2) + blk * 8, 8), 8)
        for j in range(2):
            words = [
                pltpu.pack_elementwise([src[2 * i] >> 16, src[2 * i + 1] >> 16] if j
                                       else [src[2 * i], src[2 * i + 1]],
                                       packed_dtype=jnp.uint16)
                for i in range(8)]
            for p, tile in enumerate(transpose8(words)):
                wqkv_v[grp * 8 + p, drow, pl.ds((2 * w + j) * Dh, Dh)] = tile.astype(U32)
        return wqkv_v[n_pair, pl.ds(pl.multiple_of(c * 8, 8), 8), pl.ds(0, Dh)]

    def repack_o(c, slot, i):
        orow = pl.ds(pl.multiple_of(c * (o_ch // 2) + i * (RO // 2), RO // 2), RO // 2)
        wo_v[orow, :] = pltpu.bitcast(sto_v[slot, pl.ds(i * RO, RO), :], U32)
        return wo_v[pl.ds(pl.multiple_of(H * Dh // 2 + c * 8, 8), 8), pl.ds(0, 128)]

    def phase1(c, carry):
        slot = c % 2
        for cp in stage_copies(c, slot):
            cp.wait()

        n_f = F // FC
        jobs = [functools.partial(repack_qkv, c, slot, w, blk, grp)
                for w in range(3) for blk in range(d_ch // 16) for grp in range(H // 16)]
        jobs += [functools.partial(repack_o, c, slot, i) for i in range(o_ch // RO)]
        jobs += norm3_jobs((c + 1) % n_ch)

        def share(k):
            return jobs[k * len(jobs) // (2 * n_f):(k + 1) * len(jobs) // (2 * n_f)]

        rows = chunk(c)
        u = {}
        for t in range(n_f + 1):
            if t < n_f:
                up = with_side_jobs(_dot(n3_v[rows, :], w3_v[:, pl.ds(t * FC, FC)]),
                                   share(max(2 * t - 1, 0)))
                u[t] = _gelu(up).astype(BF16)
            if t >= 1:
                down = with_side_jobs(_dot(u.pop(t - 1), w4_v[pl.ds((t - 1) * FC, FC), :]),
                                     share(min(2 * t, 2 * n_f - 1)))
                y = g_v[rows, :] + down
                if t == n_f:
                    y = y * jax.nn.sigmoid(y)
                g_v[rows, :] = y

        @pl.when(c + 2 < n_ch)
        def _():
            for cp in stage_copies(c + 2, slot):
                cp.start()

        return carry

    lax.fori_loop(0, n_ch, phase1, 0)

    L = M + SEG
    scale = Dh ** (-0.5)
    ri = lax.broadcasted_iota(jnp.int32, (2 * L, 2 * L), 0)
    ci = lax.broadcasted_iota(jnp.int32, (2 * L, 2 * L), 1)
    same_head = (ri >= L) == (ci >= L)
    rl = jnp.where(ri >= L, ri - L, ri)
    cl = jnp.where(ci >= L, ci - L, ci)
    visible = same_head & ((rl < M) | (rl >= cl))
    fill = jnp.where(same_head, F32(-1e9), F32(-jnp.inf))

    def heads_to_rows(y):
        return jnp.concatenate([y[:, :Dh], y[:, Dh:]], axis=0).astype(BF16)

    def wqkv(p):
        return pltpu.bitcast(wqkv_v[p], BF16)

    def wo(p, n):
        return pltpu.bitcast(wo_v[pl.ds(p * Dh, n * Dh), :], BF16)

    def segment(h, get_y, get_o):
        n_grp = n_pair // G
        qkv, ev, outs = {}, {}, {}
        acc = None
        for t in range(n_grp + 3):
            if t < n_grp:
                for p in range(t * G, (t + 1) * G):
                    y = get_y(p, _dot(h, wqkv(p)))
                    qkv[p] = [heads_to_rows(y[:, 2 * Dh * i:2 * Dh * (i + 1)]) for i in range(3)]
            if 0 <= t - 1 < n_grp:
                for p in range((t - 1) * G, t * G):
                    q, k, v = qkv.pop(p)
                    s = lax.dot_general(q, k, (((1,), (1,)), ((), ())), preferred_element_type=F32)
                    s = jnp.where(visible, s * scale, fill)
                    e = jnp.exp(s - jnp.max(s, axis=-1, keepdims=True))
                    l = jnp.sum(e, axis=-1, keepdims=True)
                    r = pl.reciprocal(l, approx=True)
                    ev[p] = (e.astype(BF16), v, r * (2.0 - l * r))
            if 0 <= t - 2 < n_grp:
                for p in range((t - 2) * G, (t - 1) * G):
                    e, v, r = ev.pop(p)
                    o = _dot(e, v) * r
                    o = jnp.concatenate([o[:L], o[L:]], axis=1)
                    outs[p] = get_o(p, o).astype(BF16)
            if 0 <= t - 3 < n_grp:
                p0 = (t - 3) * G
                o = jnp.concatenate([outs.pop(p) for p in range(p0, p0 + G)], axis=1)
                part = _dot(o, wo(p0, G))
                acc = part if acc is None else acc + part
        return acc

    def two_segments(j, mem):
        r0 = pl.multiple_of(j * (2 * SEG), 2 * SEG)
        rows = pl.ds(r0, 2 * SEG)
        xn = xn_v[rows, :].astype(F32)
        stash_y, stash_o = {}, {}

        def y_a(p, y):
            stash_y[p] = y[L:]
            return y[:L]

        def o_a(p, o):
            stash_o[p] = o[SEG:]
            return o[:SEG]

        acc_a = segment(jnp.concatenate([mem, xn[:L]], axis=0).astype(BF16), y_a, o_a)

        def y_b(p, y):
            return jnp.concatenate([y[:M], stash_y[p], y[M:]], axis=0)

        def o_b(p, o):
            return jnp.concatenate([o, stash_o[p]], axis=0)

        acc_b = segment(jnp.concatenate([acc_a[:M], xn[L:]], axis=0).astype(BF16), y_b, o_b)

        s = jnp.concatenate([acc_a[M:], acc_b[L:], acc_b[M:L]], axis=0)
        res = x_v[rows, :].astype(F32) + s * g_v[rows, :]
        x_v[rows, :] = res.astype(x_v.dtype)
        pltpu.make_async_copy(x_v.at[rows], out_hbm.at[rows], o_sem.at[0]).start()
        return acc_b[:M]

    lax.fori_loop(0, S // (2 * SEG), two_segments, mem0_ref[...].astype(F32))
    pltpu.make_async_copy(x_v, out_hbm, o_sem.at[0]).wait()


@functools.partial(jax.jit, static_argnames=("A_seg_len",))
def pallas_recurrent_scan__memory_aug_recurrent_mem_tr__mixer_s_mlp__prompt_kernel(
    A_x: jax.Array,
    A_mem0: jax.Array,
    A_Wq: jax.Array,
    A_Wk: jax.Array,
    A_Wv: jax.Array,
    A_Wo: jax.Array,
    A_seg_len: int,
    B_x: jax.Array,
    B_w1: jax.Array,
    B_w2: jax.Array,
    B_w3: jax.Array,
    B_w4: jax.Array,
):
    del B_x
    B, S, D = A_x.shape
    _, H, Dh = A_Wq.shape
    M = A_mem0.shape[1]
    F = B_w3.shape[1]
    SEG = int(A_seg_len)
    assert B == 1 and S % CH == 0 and S % (2 * SEG) == 0 and H % 2 == 0
    n_ch = S // CH
    d_ch = D // n_ch
    o_ch = (H * Dh) // n_ch

    any_spec = pl.BlockSpec(memory_space=pl.ANY)
    out = pl.pallas_call(
        functools.partial(_kernel, S=S, D=D, F=F, H=H, Dh=Dh, M=M, SEG=SEG),
        out_shape=jax.ShapeDtypeStruct((S, D), A_x.dtype),
        in_specs=[any_spec, pl.BlockSpec(memory_space=pltpu.VMEM)] + [any_spec] * 8,
        out_specs=any_spec,
        scratch_shapes=[
            pltpu.VMEM((S, D), BF16),
            pltpu.VMEM((S, D), BF16),
            pltpu.VMEM((S + 16 * n_ch, D), BF16),
            pltpu.VMEM((S + 16 * n_ch, D), BF16),
            pltpu.VMEM((S + 2 * HALO, D), F32),
            pltpu.VMEM((S, D), F32),
            pltpu.VMEM((D, D), BF16),
            pltpu.VMEM((D, D), BF16),
            pltpu.VMEM((D, F), BF16),
            pltpu.VMEM((F, D), BF16),
            pltpu.VMEM((2, d_ch * H, Dh), BF16),
            pltpu.VMEM((2, d_ch * H, Dh), BF16),
            pltpu.VMEM((2, d_ch * H, Dh), BF16),
            pltpu.VMEM((2, o_ch, D), BF16),
            pltpu.VMEM((H // 2 + 1, D // 2, 6 * Dh), U32),
            pltpu.VMEM((H * Dh // 2 + 8 * n_ch, D), U32),
            pltpu.SemaphoreType.DMA((n_ch,)),
            pltpu.SemaphoreType.DMA((4,)),
            pltpu.SemaphoreType.DMA((8,)),
            pltpu.SemaphoreType.DMA((1,)),
        ],
        compiler_params=pltpu.CompilerParams(vmem_limit_bytes=120 * 1024 * 1024),
    )(
        A_x.reshape(S, D),
        A_mem0.reshape(M, D),
        A_Wq.reshape(D * H, Dh),
        A_Wk.reshape(D * H, Dh),
        A_Wv.reshape(D * H, Dh),
        A_Wo.reshape(H * Dh, D),
        B_w1, B_w2, B_w3, B_w4,
    )
    return out.reshape(B, S, D)
```

```python
import functools

import jax
import jax.numpy as jnp
import numpy as np
from jax import lax
import jax.experimental.pallas as pl
import jax.experimental.pallas.tpu as pltpu

F32 = jnp.float32
BF16 = jnp.bfloat16
U32 = jnp.uint32

EPS = 1e-5
CH = 256
FC = 512
RN = 16
RO = 64
G = 2
HALO = 8


def _layernorm(x):
    m = jnp.mean(x, axis=-1, keepdims=True)
    d = x - m
    v = jnp.mean(d * d, axis=-1, keepdims=True)
    return d * lax.rsqrt(v + EPS)


def _gelu(x):
    return jax.nn.gelu(x, approximate=True)


def _dot(a, b):
    return jnp.dot(a, b, preferred_element_type=F32)


def _kernel(
    x_hbm, mem0_ref, wq_hbm, wk_hbm, wv_hbm, wo_hbm, w1_hbm, w2_hbm, w3_hbm, w4_hbm,
    out_hbm,
    x_v, xn_v, n_v, n3_v, h_v, g_v, w1_v, w2_v, w3_v, w4_v,
    stq_v, stk_v, stv_v, sto_v, wqkv_v, wo_v,
    x_sem, w_sem, st_sem, o_sem,
    *, S, D, F, H, Dh, M, SEG,
):
    n_ch = S // CH
    n_pair = H // 2
    d_ch = D // n_ch
    o_ch = (H * Dh) // n_ch
    c4 = D // 4

    def x_copy(c):
        r = pl.ds(pl.multiple_of(c * CH, CH), CH)
        return pltpu.make_async_copy(x_hbm.at[r], x_v.at[r], x_sem.at[c])

    w_copies = [
        pltpu.make_async_copy(src, dst, w_sem.at[i])
        for i, (src, dst) in enumerate(
            ((w1_hbm, w1_v), (w2_hbm, w2_v), (w3_hbm, w3_v), (w4_hbm, w4_v)))
    ]

    def stage_copies(c, slot):
        rq = pl.ds(pl.multiple_of(c * (d_ch * H), d_ch * H), d_ch * H)
        ro = pl.ds(pl.multiple_of(c * o_ch, o_ch), o_ch)
        return [
            pltpu.make_async_copy(wq_hbm.at[rq], stq_v.at[slot], st_sem.at[slot * 4 + 0]),
            pltpu.make_async_copy(wk_hbm.at[rq], stk_v.at[slot], st_sem.at[slot * 4 + 1]),
            pltpu.make_async_copy(wv_hbm.at[rq], stv_v.at[slot], st_sem.at[slot * 4 + 2]),
            pltpu.make_async_copy(wo_hbm.at[ro], sto_v.at[slot], st_sem.at[slot * 4 + 3]),
        ]

    x_copy(0).start()
    x_copy(1).start()
    w_copies[0].start()

    def chunk(c):
        return pl.ds(pl.multiple_of(c * CH, CH), CH)

    def dot_with_jobs(a, w, jobs):
        if jobs:
            w = pltpu.bitcast(w, U32)
            n_t, half = w.shape[1] // 128, w.shape[0] // 2
            cols = []
            for j in range(n_t):
                rows = []
                for i in range(2):
                    part = w[i * half:(i + 1) * half, 128 * j:128 * (j + 1)]
                    k = 2 * j + i - 1
                    if k >= 0:
                        top = part[:8]
                        for job in jobs[k * len(jobs) // (2 * n_t - 1):
                                        (k + 1) * len(jobs) // (2 * n_t - 1)]:
                            top = top | job()
                        part = jnp.concatenate([top, part[8:]], axis=0)
                    rows.append(part)
                cols.append(jnp.concatenate(rows, axis=0))
            w = pltpu.bitcast(jnp.concatenate(cols, axis=1), BF16)
        return _dot(a, w)

    def with_side_jobs(y, jobs):
        if not jobs:
            return y
        n_t = y.shape[1] // 128
        per = -(-len(jobs) // n_t)
        step = y.shape[0] // per
        cols = []
        for j in range(n_t):
            col = y[:, 128 * j:128 * (j + 1)]
            mine = jobs[j * len(jobs) // n_t:(j + 1) * len(jobs) // n_t]
            rows = []
            for i, job in enumerate(mine):
                rows += [col[i * step:i * step + 8] + pltpu.bitcast(job(), F32), col[i * step + 8:(i + 1) * step]]
            rows.append(col[len(mine) * step:])
            cols.append(jnp.concatenate([r for r in rows if r.shape[0]], axis=0))
        return jnp.concatenate(cols, axis=1)

    n_v[pl.ds(S, 16 * n_ch), pl.ds(0, 128)] = jnp.zeros((16 * n_ch, 128), BF16)
    n3_v[pl.ds(S, 16 * n_ch), pl.ds(0, 128)] = jnp.zeros((16 * n_ch, 128), BF16)
    wqkv_v[n_pair, pl.ds(0, 8 * n_ch), pl.ds(0, Dh)] = jnp.zeros((8 * n_ch, Dh), U32)
    wo_v[pl.ds(H * Dh // 2, 8 * n_ch), pl.ds(0, 128)] = jnp.zeros((8 * n_ch, 128), U32)

    h_v[pl.ds(HALO, 8), :] = jnp.zeros((8, D), F32)
    h_v[pl.ds(HALO + S - 8, 8), :] = jnp.zeros((8, D), F32)

    def norm_jobs(c):
        def job(i):
            r = pl.ds(pl.multiple_of(c * CH + i * RN, RN), RN)
            xn = _layernorm(x_v[r, :].astype(F32)).astype(BF16)
            xn_v[r, :] = xn
            n_v[r, :] = _layernorm(xn.astype(F32)).astype(BF16)
            z = n_v[pl.ds(pl.multiple_of(S + c * 16, 16), 16), pl.ds(0, 128)]
            return pltpu.bitcast(z, U32)
        return [functools.partial(job, i) for i in range(CH // RN)]

    def w1_stage(c, jobs=()):
        h = _gelu(dot_with_jobs(n_v[chunk(c), :], w1_v[...], jobs))
        win = h_v.at[pl.ds(pl.multiple_of(c * CH, CH), CH + 2 * HALO)]
        for j, sh in enumerate((-1, 1, -2, 2)):
            win[pl.ds(HALO - sh, CH), pl.ds(j * c4, c4)] = h[:, j * c4:(j + 1) * c4]

    def w2_stage(c, jobs=()):
        hs = h_v[pl.ds(pl.multiple_of(c * CH + HALO, HALO), CH), :].astype(BF16)
        g_v[chunk(c), :] = xn_v[chunk(c), :].astype(F32) + dot_with_jobs(hs, w2_v[...], jobs)

    def norm3_jobs(c):
        def job(i):
            r = pl.ds(pl.multiple_of(c * CH + i * RN, RN), RN)
            n3_v[r, :] = _layernorm(g_v[r, :]).astype(BF16)
            z = n3_v[pl.ds(pl.multiple_of(S + c * 16, 16), 16), pl.ds(0, 128)]
            return pltpu.bitcast(z, U32)
        return [functools.partial(job, i) for i in range(CH // RN)]

    x_copy(0).wait()
    for job in norm_jobs(0):
        job()
    x_copy(1).wait()
    for job in norm_jobs(1)[:CH // RN // 2]:
        job()
    w_copies[0].wait()
    x_copy(2).start()
    w_copies[1].start()

    @pl.loop(0, n_ch + 2)
    def _(c):
        @pl.when(c == 1)
        def _():
            for i in range(3, n_ch):
                x_copy(i).start()

        @pl.when(c == 2)
        def _():
            w_copies[1].wait()
            for cp in w_copies[2:] + stage_copies(0, 0) + stage_copies(1, 1):
                cp.start()

        @pl.when((c >= 1) & (c + 1 < n_ch))
        def _():
            x_copy(c + 1).wait()

        jobs = norm_jobs(jnp.minimum(c + 1, n_ch - 1))
        half = len(jobs) // 2

        @pl.when(c == 1)
        def _():
            for job in jobs[:half]:
                job()

        @pl.when(c >= 2)
        def _():
            w2_stage(c - 2, jobs[:half])

        @pl.when(c < n_ch)
        def _():
            w1_stage(c, jobs[half:])

    for job in norm3_jobs(0):
        job()

    for cp in w_copies[2:]:
        cp.wait()

    sub = lax.broadcasted_iota(jnp.int32, (8, Dh), 0)

    def transpose8(vs):
        for s in (4, 2, 1):
            upper = (sub & s) != 0
            out = list(vs)
            for i in range(8):
                if not i & s:
                    a, b = vs[i], vs[i + s]
                    out[i] = jnp.where(upper, pltpu.roll(b, s, 0), a)
                    out[i + s] = jnp.where(upper, b, pltpu.roll(a, 8 - s, 0))
            vs = out
        return vs

    def repack_qkv(c, slot, w, blk, grp):
        st = (stq_v, stk_v, stv_v)[w]
        src = [pltpu.bitcast(st[slot, pl.ds((blk * 16 + d) * H + grp * 16, 16), :], U32)
               for d in range(16)]
        drow = pl.ds(pl.multiple_of(c * (d_ch // 2) + blk * 8, 8), 8)
        for j in range(2):
            words = [
                pltpu.pack_elementwise([src[2 * i] >> 16, src[2 * i + 1] >> 16] if j
                                       else [src[2 * i], src[2 * i + 1]],
                                       packed_dtype=jnp.uint16)
                for i in range(8)]
            for p, tile in enumerate(transpose8(words)):
                wqkv_v[grp * 8 + p, drow, pl.ds((2 * w + j) * Dh, Dh)] = tile.astype(U32)
        return wqkv_v[n_pair, pl.ds(pl.multiple_of(c * 8, 8), 8), pl.ds(0, Dh)]

    def repack_o(c, slot, i):
        orow = pl.ds(pl.multiple_of(c * (o_ch // 2) + i * (RO // 2), RO // 2), RO // 2)
        wo_v[orow, :] = pltpu.bitcast(sto_v[slot, pl.ds(i * RO, RO), :], U32)
        return wo_v[pl.ds(pl.multiple_of(H * Dh // 2 + c * 8, 8), 8), pl.ds(0, 128)]

    def phase1(c, carry):
        slot = c % 2
        for cp in stage_copies(c, slot):
            cp.wait()

        n_f = F // FC
        jobs = [functools.partial(repack_qkv, c, slot, w, blk, grp)
                for w in range(3) for blk in range(d_ch // 16) for grp in range(H // 16)]
        jobs += [functools.partial(repack_o, c, slot, i) for i in range(o_ch // RO)]
        jobs += norm3_jobs((c + 1) % n_ch)

        def share(k):
            return jobs[k * len(jobs) // (2 * n_f):(k + 1) * len(jobs) // (2 * n_f)]

        rows = chunk(c)
        u = {}
        for t in range(n_f + 1):
            if t < n_f:
                up = with_side_jobs(_dot(n3_v[rows, :], w3_v[:, pl.ds(t * FC, FC)]),
                                   share(max(2 * t - 1, 0)))
                u[t] = _gelu(up).astype(BF16)
            if t >= 1:
                down = with_side_jobs(_dot(u.pop(t - 1), w4_v[pl.ds((t - 1) * FC, FC), :]),
                                     share(min(2 * t, 2 * n_f - 1)))
                y = g_v[rows, :] + down
                g_v[rows, :] = y

        @pl.when(c + 2 < n_ch)
        def _():
            for cp in stage_copies(c + 2, slot):
                cp.start()

        return carry

    lax.fori_loop(0, n_ch, phase1, 0)

    L = M + SEG
    scale = Dh ** (-0.5)
    ri = lax.broadcasted_iota(jnp.int32, (2 * L, 2 * L), 0)
    ci = lax.broadcasted_iota(jnp.int32, (2 * L, 2 * L), 1)
    same_head = (ri >= L) == (ci >= L)
    rl = jnp.where(ri >= L, ri - L, ri)
    cl = jnp.where(ci >= L, ci - L, ci)
    visible = same_head & ((rl < M) | (rl >= cl))
    fill = jnp.where(same_head, F32(-1e9), F32(-jnp.inf))

    def heads_to_rows(y):
        return jnp.concatenate([y[:, :Dh], y[:, Dh:]], axis=0).astype(BF16)

    def wqkv(p):
        return pltpu.bitcast(wqkv_v[p], BF16)

    def wo(p, n):
        return pltpu.bitcast(wo_v[pl.ds(p * Dh, n * Dh), :], BF16)

    def segment(h, get_y, get_o):
        n_grp = n_pair // G
        qkv, ev, outs = {}, {}, {}
        acc = None
        for t in range(n_grp + 3):
            if t < n_grp:
                for p in range(t * G, (t + 1) * G):
                    y = get_y(p, _dot(h, wqkv(p)))
                    qkv[p] = [heads_to_rows(y[:, 2 * Dh * i:2 * Dh * (i + 1)]) for i in range(3)]
            if 0 <= t - 1 < n_grp:
                for p in range((t - 1) * G, t * G):
                    q, k, v = qkv.pop(p)
                    s = lax.dot_general(q, k, (((1,), (1,)), ((), ())), preferred_element_type=F32)
                    s = jnp.where(visible, s * scale, fill)
                    e = jnp.exp(s - jnp.max(s, axis=-1, keepdims=True))
                    l = jnp.sum(e, axis=-1, keepdims=True)
                    r = pl.reciprocal(l, approx=True)
                    ev[p] = (e.astype(BF16), v, r * (2.0 - l * r))
            if 0 <= t - 2 < n_grp:
                for p in range((t - 2) * G, (t - 1) * G):
                    e, v, r = ev.pop(p)
                    o = _dot(e, v) * r
                    o = jnp.concatenate([o[:L], o[L:]], axis=1)
                    outs[p] = get_o(p, o).astype(BF16)
            if 0 <= t - 3 < n_grp:
                p0 = (t - 3) * G
                o = jnp.concatenate([outs.pop(p) for p in range(p0, p0 + G)], axis=1)
                part = _dot(o, wo(p0, G))
                acc = part if acc is None else acc + part
        return acc

    def two_segments(j, mem):
        r0 = pl.multiple_of(j * (2 * SEG), 2 * SEG)
        rows = pl.ds(r0, 2 * SEG)
        xn = xn_v[rows, :].astype(F32)
        stash_y, stash_o = {}, {}

        def y_a(p, y):
            stash_y[p] = y[L:]
            return y[:L]

        def o_a(p, o):
            stash_o[p] = o[SEG:]
            return o[:SEG]

        acc_a = segment(jnp.concatenate([mem, xn[:L]], axis=0).astype(BF16), y_a, o_a)

        def y_b(p, y):
            return jnp.concatenate([y[:M], stash_y[p], y[M:]], axis=0)

        def o_b(p, o):
            return jnp.concatenate([o, stash_o[p]], axis=0)

        acc_b = segment(jnp.concatenate([acc_a[:M], xn[L:]], axis=0).astype(BF16), y_b, o_b)

        s = jnp.concatenate([acc_a[M:], acc_b[L:], acc_b[M:L]], axis=0)
        res = x_v[rows, :].astype(F32) + s * jax.nn.silu(g_v[rows, :])
        x_v[rows, :] = res.astype(x_v.dtype)
        pltpu.make_async_copy(x_v.at[rows], out_hbm.at[rows], o_sem.at[0]).start()
        return acc_b[:M]

    lax.fori_loop(0, S // (2 * SEG), two_segments, mem0_ref[...].astype(F32))
    pltpu.make_async_copy(x_v, out_hbm, o_sem.at[0]).wait()


@functools.partial(jax.jit, static_argnames=("A_seg_len",))
def pallas_recurrent_scan__memory_aug_recurrent_mem_tr__mixer_s_mlp__prompt_kernel(
    A_x: jax.Array,
    A_mem0: jax.Array,
    A_Wq: jax.Array,
    A_Wk: jax.Array,
    A_Wv: jax.Array,
    A_Wo: jax.Array,
    A_seg_len: int,
    B_x: jax.Array,
    B_w1: jax.Array,
    B_w2: jax.Array,
    B_w3: jax.Array,
    B_w4: jax.Array,
):
    del B_x
    B, S, D = A_x.shape
    _, H, Dh = A_Wq.shape
    M = A_mem0.shape[1]
    F = B_w3.shape[1]
    SEG = int(A_seg_len)
    assert B == 1 and S % CH == 0 and S % (2 * SEG) == 0 and H % 2 == 0
    n_ch = S // CH
    d_ch = D // n_ch
    o_ch = (H * Dh) // n_ch

    any_spec = pl.BlockSpec(memory_space=pl.ANY)
    out = pl.pallas_call(
        functools.partial(_kernel, S=S, D=D, F=F, H=H, Dh=Dh, M=M, SEG=SEG),
        out_shape=jax.ShapeDtypeStruct((S, D), A_x.dtype),
        in_specs=[any_spec, pl.BlockSpec(memory_space=pltpu.VMEM)] + [any_spec] * 8,
        out_specs=any_spec,
        scratch_shapes=[
            pltpu.VMEM((S, D), BF16),
            pltpu.VMEM((S, D), BF16),
            pltpu.VMEM((S + 16 * n_ch, D), BF16),
            pltpu.VMEM((S + 16 * n_ch, D), BF16),
            pltpu.VMEM((S + 2 * HALO, D), F32),
            pltpu.VMEM((S, D), F32),
            pltpu.VMEM((D, D), BF16),
            pltpu.VMEM((D, D), BF16),
            pltpu.VMEM((D, F), BF16),
            pltpu.VMEM((F, D), BF16),
            pltpu.VMEM((2, d_ch * H, Dh), BF16),
            pltpu.VMEM((2, d_ch * H, Dh), BF16),
            pltpu.VMEM((2, d_ch * H, Dh), BF16),
            pltpu.VMEM((2, o_ch, D), BF16),
            pltpu.VMEM((H // 2 + 1, D // 2, 6 * Dh), U32),
            pltpu.VMEM((H * Dh // 2 + 8 * n_ch, D), U32),
            pltpu.SemaphoreType.DMA((n_ch,)),
            pltpu.SemaphoreType.DMA((4,)),
            pltpu.SemaphoreType.DMA((8,)),
            pltpu.SemaphoreType.DMA((1,)),
        ],
        compiler_params=pltpu.CompilerParams(vmem_limit_bytes=120 * 1024 * 1024),
    )(
        A_x.reshape(S, D),
        A_mem0.reshape(M, D),
        A_Wq.reshape(D * H, Dh),
        A_Wk.reshape(D * H, Dh),
        A_Wv.reshape(D * H, Dh),
        A_Wo.reshape(H * Dh, D),
        B_w1, B_w2, B_w3, B_w4,
    )
    return out.reshape(B, S, D)
```

```python
import functools

import jax
import jax.numpy as jnp
import numpy as np
from jax import lax
import jax.experimental.pallas as pl
import jax.experimental.pallas.tpu as pltpu

F32 = jnp.float32
BF16 = jnp.bfloat16
U32 = jnp.uint32

EPS = 1e-5
CH = 256
FC = 512
RN = 16
RO = 64
G = 2
HALO = 8
SHIFTS = (-1, 1, -2, 2)


def _layernorm(x):
    m = jnp.mean(x, axis=-1, keepdims=True)
    d = x - m
    v = jnp.mean(d * d, axis=-1, keepdims=True)
    return d * lax.rsqrt(v + EPS)


def _gelu(x):
    return jax.nn.gelu(x, approximate=True)


def _dot(a, b):
    return jnp.dot(a, b, preferred_element_type=F32)


def _dot_with_jobs(a, w, jobs):
    w = pltpu.bitcast(w, U32)
    n_t, half = w.shape[1] // 128, w.shape[0] // 2
    n_due = 2 * n_t - 1
    cols = []
    for j in range(n_t):
        rows = []
        for i in range(2):
            part = w[i * half:(i + 1) * half, 128 * j:128 * (j + 1)]
            k = 2 * j + i - 1
            if k >= 0:
                top = part[:8]
                for job in jobs[k * len(jobs) // n_due:(k + 1) * len(jobs) // n_due]:
                    top = top | job()
                part = jnp.concatenate([top, part[8:]], axis=0)
            rows.append(part)
        cols.append(jnp.concatenate(rows, axis=0))
    return _dot(a, pltpu.bitcast(jnp.concatenate(cols, axis=1), BF16))


def _jobs_before_use(y, jobs):
    n_t = y.shape[1] // 128
    step = y.shape[0] // -(-len(jobs) // n_t)
    cols = []
    for j in range(n_t):
        col = y[:, 128 * j:128 * (j + 1)]
        mine = jobs[j * len(jobs) // n_t:(j + 1) * len(jobs) // n_t]
        rows = []
        for i, job in enumerate(mine):
            rows.append(col[i * step:i * step + 8] + pltpu.bitcast(job(), F32))
            rows.append(col[i * step + 8:(i + 1) * step])
        rows.append(col[len(mine) * step:])
        cols.append(jnp.concatenate([r for r in rows if r.shape[0]], axis=0))
    return jnp.concatenate(cols, axis=1)


def _transpose8(vs):
    sub = lax.broadcasted_iota(jnp.int32, vs[0].shape, 0)
    for s in (4, 2, 1):
        upper = (sub & s) != 0
        out = list(vs)
        for i in range(8):
            if not i & s:
                a, b = vs[i], vs[i + s]
                out[i] = jnp.where(upper, pltpu.roll(b, s, 0), a)
                out[i + s] = jnp.where(upper, b, pltpu.roll(a, 8 - s, 0))
        vs = out
    return vs


def _kernel(
    x_hbm, mem0_hbm, wq_hbm, wk_hbm, wv_hbm, wo_hbm, w1_hbm, w2_hbm, w3_hbm, w4_hbm,
    out_hbm,
    x_v, xn_v, n_v, n3_v, h_v, y_v, mem0_v, w1_v, w2_v, w3_v, w4_v,
    stq_v, stk_v, stv_v, sto_v, wqkv_v, wo_v,
    x_sem, w_sem, st_sem, o_sem,
    *, S, D, F, H, Dh, M, SEG,
):
    n_ch = S // CH
    n_pair = H // 2
    d_ch = D // n_ch
    o_ch = (H * Dh) // n_ch
    c4 = D // 4

    def chunk(c):
        return pl.ds(pl.multiple_of(c * CH, CH), CH)

    def x_copy(c):
        return pltpu.make_async_copy(x_hbm.at[chunk(c)], x_v.at[chunk(c)], x_sem.at[c])

    w1_copy, w2_copy, *late_copies = [
        pltpu.make_async_copy(src, dst, w_sem.at[i])
        for i, (src, dst) in enumerate((
            (w1_hbm, w1_v), (w2_hbm, w2_v), (w3_hbm, w3_v), (w4_hbm, w4_v), (mem0_hbm, mem0_v)))
    ]

    def stage_copies(c, slot):
        rq = pl.ds(pl.multiple_of(c * (d_ch * H), d_ch * H), d_ch * H)
        ro = pl.ds(pl.multiple_of(c * o_ch, o_ch), o_ch)
        return [
            pltpu.make_async_copy(src, dst.at[slot], st_sem.at[slot * 4 + i])
            for i, (src, dst) in enumerate((
                (wq_hbm.at[rq], stq_v), (wk_hbm.at[rq], stk_v),
                (wv_hbm.at[rq], stv_v), (wo_hbm.at[ro], sto_v)))
        ]

    x_copy(0).start()
    x_copy(1).start()
    w1_copy.start()

    n_v[pl.ds(S, 16 * n_ch), pl.ds(0, 128)] = jnp.zeros((16 * n_ch, 128), BF16)
    n3_v[pl.ds(S, 16 * n_ch), pl.ds(0, 128)] = jnp.zeros((16 * n_ch, 128), BF16)
    wqkv_v[n_pair, pl.ds(0, 8 * n_ch), pl.ds(0, 128)] = jnp.zeros((8 * n_ch, 128), U32)
    wo_v[pl.ds(H * Dh // 2, 8 * n_ch), pl.ds(0, 128)] = jnp.zeros((8 * n_ch, 128), U32)

    h_v[pl.ds(HALO, 8), :] = jnp.zeros((8, D), F32)
    h_v[pl.ds(HALO + S - 8, 8), :] = jnp.zeros((8, D), F32)

    def zero_tile(ref, c):
        return pltpu.bitcast(ref[pl.ds(pl.multiple_of(S + c * 16, 16), 16), pl.ds(0, 128)], U32)

    def norm_jobs(c):
        def job(i):
            r = pl.ds(pl.multiple_of(c * CH + i * RN, RN), RN)
            xn = _layernorm(x_v[r, :].astype(F32)).astype(BF16)
            xn_v[r, :] = xn
            n_v[r, :] = _layernorm(xn.astype(F32)).astype(BF16)
            return zero_tile(n_v, c)
        return [functools.partial(job, i) for i in range(CH // RN)]

    def norm3_jobs(c):
        def job(i):
            r = pl.ds(pl.multiple_of(c * CH + i * RN, RN), RN)
            n3_v[r, :] = _layernorm(y_v[r, :]).astype(BF16)
            return zero_tile(n3_v, c)
        return [functools.partial(job, i) for i in range(CH // RN)]

    def w1_stage(c, jobs):
        h = _gelu(_dot_with_jobs(n_v[chunk(c), :], w1_v[...], jobs))
        win = h_v.at[pl.ds(pl.multiple_of(c * CH, CH), CH + 2 * HALO)]
        for j, sh in enumerate(SHIFTS):
            win[pl.ds(HALO - sh, CH), pl.ds(j * c4, c4)] = h[:, j * c4:(j + 1) * c4]

    def w2_stage(c, jobs):
        hs = h_v[pl.ds(pl.multiple_of(c * CH + HALO, HALO), CH), :].astype(BF16)
        y_v[chunk(c), :] = xn_v[chunk(c), :].astype(F32) + _dot_with_jobs(hs, w2_v[...], jobs)

    half = CH // RN // 2
    x_copy(0).wait()
    for job in norm_jobs(0):
        job()
    x_copy(1).wait()
    for job in norm_jobs(1)[:half]:
        job()
    w1_copy.wait()
    x_copy(2).start()
    w2_copy.start()

    @pl.loop(0, n_ch + 2)
    def _(c):
        @pl.when(c == 1)
        def _():
            for i in range(3, n_ch):
                x_copy(i).start()

        @pl.when(c == 2)
        def _():
            w2_copy.wait()
            for cp in late_copies + stage_copies(0, 0) + stage_copies(1, 1):
                cp.start()

        @pl.when((c >= 1) & (c + 1 < n_ch))
        def _():
            x_copy(c + 1).wait()

        jobs = norm_jobs(jnp.minimum(c + 1, n_ch - 1))

        @pl.when(c == 1)
        def _():
            for job in jobs[:half]:
                job()

        @pl.when(c >= 2)
        def _():
            w2_stage(c - 2, jobs[:half])

        @pl.when(c < n_ch)
        def _():
            w1_stage(c, jobs[half:])

    for job in norm3_jobs(0):
        job()

    for cp in late_copies:
        cp.wait()

    def repack_qkv(c, slot, w, blk, grp):
        st = (stq_v, stk_v, stv_v)[w]
        src = [pltpu.bitcast(st[slot, pl.ds((blk * 16 + d) * H + grp * 16, 16), :], U32)
               for d in range(16)]
        drow = pl.ds(pl.multiple_of(c * (d_ch // 2) + blk * 8, 8), 8)
        for j in range(2):
            words = [(a >> 16) | (b & np.uint32(0xFFFF0000)) if j
                     else (a & np.uint32(0xFFFF)) | (b << 16)
                     for a, b in zip(src[0::2], src[1::2])]
            for p, tile in enumerate(_transpose8(words)):
                wqkv_v[grp * 8 + p, drow, pl.ds((2 * w + j) * Dh, Dh)] = tile
        return wqkv_v[n_pair, pl.ds(pl.multiple_of(c * 8, 8), 8), pl.ds(0, 128)]

    def repack_o(c, slot, i):
        orow = pl.ds(pl.multiple_of(c * (o_ch // 2) + i * (RO // 2), RO // 2), RO // 2)
        wo_v[orow, :] = pltpu.bitcast(sto_v[slot, pl.ds(i * RO, RO), :], U32)
        return wo_v[pl.ds(pl.multiple_of(H * Dh // 2 + c * 8, 8), 8), pl.ds(0, 128)]

    @pl.loop(0, n_ch)
    def _(c):
        slot = c % 2
        for cp in stage_copies(c, slot):
            cp.wait()

        n_f = F // FC
        jobs = [functools.partial(repack_qkv, c, slot, w, blk, grp)
                for w in range(3) for blk in range(d_ch // 16) for grp in range(H // 16)]
        jobs += [functools.partial(repack_o, c, slot, i) for i in range(o_ch // RO)]
        jobs += norm3_jobs((c + 1) % n_ch)

        def share(k):
            return jobs[k * len(jobs) // (2 * n_f):(k + 1) * len(jobs) // (2 * n_f)]

        rows = chunk(c)
        u = {}
        for t in range(n_f + 1):
            if t < n_f:
                up = _dot(n3_v[rows, :], w3_v[:, pl.ds(t * FC, FC)])
                u[t] = _gelu(_jobs_before_use(up, share(max(2 * t - 1, 0)))).astype(BF16)
            if t >= 1:
                down = _dot(u.pop(t - 1), w4_v[pl.ds((t - 1) * FC, FC), :])
                down = _jobs_before_use(down, share(min(2 * t, 2 * n_f - 1)))
                y_v[rows, :] = y_v[rows, :] + down

        @pl.when(c + 2 < n_ch)
        def _():
            for cp in stage_copies(c + 2, slot):
                cp.start()

    L = M + SEG
    scale = Dh ** (-0.5)
    ri = lax.broadcasted_iota(jnp.int32, (2 * L, 2 * L), 0)
    ci = lax.broadcasted_iota(jnp.int32, (2 * L, 2 * L), 1)
    same_head = (ri >= L) == (ci >= L)
    rl = jnp.where(ri >= L, ri - L, ri)
    cl = jnp.where(ci >= L, ci - L, ci)
    visible = same_head & ((rl < M) | (rl >= cl))
    fill = jnp.where(same_head, np.float32(-1e9), np.float32(-np.inf))

    def heads_to_rows(y):
        return jnp.concatenate([y[:, :Dh], y[:, Dh:]], axis=0).astype(BF16)

    def segment(h, get_qkv, get_o):
        n_grp = n_pair // G
        qkv, probs, outs = {}, {}, {}
        acc = None
        for t in range(n_grp + 3):
            if t < n_grp:
                for p in range(t * G, (t + 1) * G):
                    y = get_qkv(p, _dot(h, pltpu.bitcast(wqkv_v[p], BF16)))
                    qkv[p] = [heads_to_rows(y[:, 2 * Dh * i:2 * Dh * (i + 1)]) for i in range(3)]
            if 0 <= t - 1 < n_grp:
                for p in range((t - 1) * G, t * G):
                    q, k, v = qkv.pop(p)
                    s = lax.dot_general(q, k, (((1,), (1,)), ((), ())),
                                        preferred_element_type=F32)
                    s = jnp.where(visible, s * scale, fill)
                    e = jnp.exp(s - jnp.max(s, axis=-1, keepdims=True))
                    l = jnp.sum(e, axis=-1, keepdims=True)
                    r = pl.reciprocal(l, approx=True)
                    probs[p] = (e.astype(BF16), v, r * (2.0 - l * r))
            if 0 <= t - 2 < n_grp:
                for p in range((t - 2) * G, (t - 1) * G):
                    e, v, r = probs.pop(p)
                    o = _dot(e, v) * r
                    outs[p] = get_o(p, jnp.concatenate([o[:L], o[L:]], axis=1)).astype(BF16)
            if 0 <= t - 3 < n_grp:
                p0 = (t - 3) * G
                o = jnp.concatenate([outs.pop(p) for p in range(p0, p0 + G)], axis=1)
                part = _dot(o, pltpu.bitcast(wo_v[pl.ds(p0 * Dh, G * Dh), :], BF16))
                acc = part if acc is None else acc + part
        return acc

    def two_segments(j, mem):
        rows = pl.ds(pl.multiple_of(j * (2 * SEG), 2 * SEG), 2 * SEG)
        xn = xn_v[rows, :].astype(F32)
        early_qkv, late_o = {}, {}

        def qkv_a(p, y):
            early_qkv[p] = y[L:]
            return y[:L]

        def o_a(p, o):
            late_o[p] = o[SEG:]
            return o[:SEG]

        def qkv_b(p, y):
            return jnp.concatenate([y[:M], early_qkv[p], y[M:]], axis=0)

        def o_b(p, o):
            return jnp.concatenate([o, late_o[p]], axis=0)

        acc_a = segment(jnp.concatenate([mem, xn[:L]], axis=0).astype(BF16), qkv_a, o_a)
        acc_b = segment(jnp.concatenate([acc_a[:M], xn[L:]], axis=0).astype(BF16), qkv_b, o_b)

        s = jnp.concatenate([acc_a[M:], acc_b[L:], acc_b[M:L]], axis=0)
        res = x_v[rows, :].astype(F32) + s * jax.nn.silu(y_v[rows, :])
        x_v[rows, :] = res.astype(x_v.dtype)
        pltpu.make_async_copy(x_v.at[rows], out_hbm.at[rows], o_sem.at[0]).start()
        return acc_b[:M]

    lax.fori_loop(0, S // (2 * SEG), two_segments, mem0_v[...].astype(F32))
    pltpu.make_async_copy(x_v, out_hbm, o_sem.at[0]).wait()


@functools.partial(jax.jit, static_argnames=("A_seg_len",))
def pallas_recurrent_scan__memory_aug_recurrent_mem_tr__mixer_s_mlp__prompt_kernel(
    A_x: jax.Array,
    A_mem0: jax.Array,
    A_Wq: jax.Array,
    A_Wk: jax.Array,
    A_Wv: jax.Array,
    A_Wo: jax.Array,
    A_seg_len: int,
    B_x: jax.Array,
    B_w1: jax.Array,
    B_w2: jax.Array,
    B_w3: jax.Array,
    B_w4: jax.Array,
):
    del B_x
    B, S, D = A_x.shape
    _, H, Dh = A_Wq.shape
    M = A_mem0.shape[1]
    F = B_w3.shape[1]
    SEG = int(A_seg_len)
    n_ch = S // CH
    d_ch = D // n_ch
    o_ch = (H * Dh) // n_ch
    assert B == 1 and S % CH == 0 and S % (2 * SEG) == 0 and F % FC == 0 and n_ch >= 4
    assert H % 16 == 0 and Dh == 128 and d_ch % 16 == 0 and M % 8 == 0 and SEG % 16 == 0

    any_spec = pl.BlockSpec(memory_space=pl.ANY)
    out = pl.pallas_call(
        functools.partial(_kernel, S=S, D=D, F=F, H=H, Dh=Dh, M=M, SEG=SEG),
        out_shape=jax.ShapeDtypeStruct((S, D), A_x.dtype),
        in_specs=[any_spec] * 10,
        out_specs=any_spec,
        scratch_shapes=[
            pltpu.VMEM((S, D), BF16),
            pltpu.VMEM((S, D), BF16),
            pltpu.VMEM((S + 16 * n_ch, D), BF16),
            pltpu.VMEM((S + 16 * n_ch, D), BF16),
            pltpu.VMEM((S + 2 * HALO, D), F32),
            pltpu.VMEM((S, D), F32),
            pltpu.VMEM((M, D), BF16),
            pltpu.VMEM((D, D), BF16),
            pltpu.VMEM((D, D), BF16),
            pltpu.VMEM((D, F), BF16),
            pltpu.VMEM((F, D), BF16),
            pltpu.VMEM((2, d_ch * H, Dh), BF16),
            pltpu.VMEM((2, d_ch * H, Dh), BF16),
            pltpu.VMEM((2, d_ch * H, Dh), BF16),
            pltpu.VMEM((2, o_ch, D), BF16),
            pltpu.VMEM((H // 2 + 1, D // 2, 6 * Dh), U32),
            pltpu.VMEM((H * Dh // 2 + 8 * n_ch, D), U32),
            pltpu.SemaphoreType.DMA((n_ch,)),
            pltpu.SemaphoreType.DMA((5,)),
            pltpu.SemaphoreType.DMA((8,)),
            pltpu.SemaphoreType.DMA((1,)),
        ],
        compiler_params=pltpu.CompilerParams(vmem_limit_bytes=120 * 1024 * 1024),
    )(
        A_x.reshape(S, D),
        A_mem0.reshape(M, D),
        A_Wq.reshape(D * H, Dh),
        A_Wk.reshape(D * H, Dh),
        A_Wv.reshape(D * H, Dh),
        A_Wo.reshape(H * Dh, D),
        B_w1, B_w2, B_w3, B_w4,
    )
    return out.reshape(B, S, D)
```

```python
import functools

import jax
import jax.numpy as jnp
import numpy as np
from jax import lax
import jax.experimental.pallas as pl
import jax.experimental.pallas.tpu as pltpu

F32 = jnp.float32
BF16 = jnp.bfloat16
U32 = jnp.uint32

EPS = 1e-5
CH = 256
FC = 512
RN = 16
RO = 64
G = 2
HALO = 8
SHIFTS = (-1, 1, -2, 2)


def _layernorm(x):
    m = jnp.mean(x, axis=-1, keepdims=True)
    d = x - m
    v = jnp.mean(d * d, axis=-1, keepdims=True)
    return d * lax.rsqrt(v + EPS)


def _gelu(x):
    return jax.nn.gelu(x, approximate=True)


def _dot(a, b):
    return jnp.dot(a, b, preferred_element_type=F32)


def _dot_with_jobs(a, w, jobs):
    w = pltpu.bitcast(w, U32)
    n_t, half = w.shape[1] // 128, w.shape[0] // 2
    n_due = 2 * n_t - 1
    cols = []
    for j in range(n_t):
        rows = []
        for i in range(2):
            part = w[i * half:(i + 1) * half, 128 * j:128 * (j + 1)]
            k = 2 * j + i - 1
            if k >= 0:
                top = part[:8]
                for job in jobs[k * len(jobs) // n_due:(k + 1) * len(jobs) // n_due]:
                    top = top | job()
                part = jnp.concatenate([top, part[8:]], axis=0)
            rows.append(part)
        cols.append(jnp.concatenate(rows, axis=0))
    return _dot(a, pltpu.bitcast(jnp.concatenate(cols, axis=1), BF16))


def _jobs_before_use(y, jobs):
    n_t = y.shape[1] // 128
    step = y.shape[0] // -(-len(jobs) // n_t)
    cols = []
    for j in range(n_t):
        col = y[:, 128 * j:128 * (j + 1)]
        mine = jobs[j * len(jobs) // n_t:(j + 1) * len(jobs) // n_t]
        rows = []
        for i, job in enumerate(mine):
            rows.append(col[i * step:i * step + 8] + pltpu.bitcast(job(), F32))
            rows.append(col[i * step + 8:(i + 1) * step])
        rows.append(col[len(mine) * step:])
        cols.append(jnp.concatenate([r for r in rows if r.shape[0]], axis=0))
    return jnp.concatenate(cols, axis=1)


def _transpose8(vs):
    sub = lax.broadcasted_iota(jnp.int32, vs[0].shape, 0)
    for s in (4, 2, 1):
        upper = (sub & s) != 0
        out = list(vs)
        for i in range(8):
            if not i & s:
                a, b = vs[i], vs[i + s]
                out[i] = jnp.where(upper, pltpu.roll(b, s, 0), a)
                out[i + s] = jnp.where(upper, b, pltpu.roll(a, 8 - s, 0))
        vs = out
    return vs


def _kernel(
    x_hbm, mem0_hbm, wq_hbm, wk_hbm, wv_hbm, wo_hbm, w1_hbm, w2_hbm, w3_hbm, w4_hbm,
    out_hbm,
    x_v, xn_v, n_v, n3_v, h_v, y_v, mem0_v, w1_v, w2_v, w3_v, w4_v,
    stq_v, stk_v, stv_v, sto_v, wqkv_v, wo_v,
    x_sem, w_sem, st_sem, o_sem,
    *, S, D, F, H, Dh, M, SEG,
):
    n_ch = S // CH
    n_pair = H // 2
    d_ch = D // n_ch
    o_ch = (H * Dh) // n_ch
    c4 = D // 4

    def chunk(c):
        return pl.ds(pl.multiple_of(c * CH, CH), CH)

    def x_copy(c):
        return pltpu.make_async_copy(x_hbm.at[chunk(c)], x_v.at[chunk(c)], x_sem.at[c])

    left, right = pl.ds(0, D // 2), pl.ds(D // 2, D // 2)
    w1_left_copy, w1_right_copy, w2_copy, *late_copies = [
        pltpu.make_async_copy(src, dst, w_sem.at[i])
        for i, (src, dst) in enumerate((
            (w1_hbm.at[:, left], w1_v.at[:, left]), (w1_hbm.at[:, right], w1_v.at[:, right]),
            (w2_hbm, w2_v), (w3_hbm, w3_v), (w4_hbm, w4_v), (mem0_hbm, mem0_v)))
    ]

    def stage_copies(c, slot):
        rq = pl.ds(pl.multiple_of(c * (d_ch * H), d_ch * H), d_ch * H)
        ro = pl.ds(pl.multiple_of(c * o_ch, o_ch), o_ch)
        return [
            pltpu.make_async_copy(src, dst.at[slot], st_sem.at[slot * 4 + i])
            for i, (src, dst) in enumerate((
                (wq_hbm.at[rq], stq_v), (wk_hbm.at[rq], stk_v),
                (wv_hbm.at[rq], stv_v), (wo_hbm.at[ro], sto_v)))
        ]

    for cp in (x_copy(0), w1_left_copy, x_copy(1), w1_right_copy):
        cp.start()

    n_v[pl.ds(S, 16 * n_ch), pl.ds(0, 128)] = jnp.zeros((16 * n_ch, 128), BF16)
    n3_v[pl.ds(S, 16 * n_ch), pl.ds(0, 128)] = jnp.zeros((16 * n_ch, 128), BF16)
    wqkv_v[n_pair, pl.ds(0, 8 * n_ch), pl.ds(0, 128)] = jnp.zeros((8 * n_ch, 128), U32)
    wo_v[pl.ds(H * Dh // 2, 8 * n_ch), pl.ds(0, 128)] = jnp.zeros((8 * n_ch, 128), U32)

    h_v[pl.ds(HALO, 8), :] = jnp.zeros((8, D), F32)
    h_v[pl.ds(HALO + S - 8, 8), :] = jnp.zeros((8, D), F32)

    def zero_tile(ref, c):
        return pltpu.bitcast(ref[pl.ds(pl.multiple_of(S + c * 16, 16), 16), pl.ds(0, 128)], U32)

    def norm_jobs(c):
        def job(i):
            r = pl.ds(pl.multiple_of(c * CH + i * RN, RN), RN)
            xn = _layernorm(x_v[r, :].astype(F32)).astype(BF16)
            xn_v[r, :] = xn
            n_v[r, :] = _layernorm(xn.astype(F32)).astype(BF16)
            return zero_tile(n_v, c)
        return [functools.partial(job, i) for i in range(CH // RN)]

    def norm3_jobs(c):
        def job(i):
            r = pl.ds(pl.multiple_of(c * CH + i * RN, RN), RN)
            n3_v[r, :] = _layernorm(y_v[r, :]).astype(BF16)
            return zero_tile(n3_v, c)
        return [functools.partial(job, i) for i in range(CH // RN)]

    def w1_stage(c, jobs, j0=0, j1=4):
        w1 = w1_v[:, pl.ds(j0 * c4, (j1 - j0) * c4)]
        h = _gelu(_dot_with_jobs(n_v[chunk(c), :], w1, jobs))
        win = h_v.at[pl.ds(pl.multiple_of(c * CH, CH), CH + 2 * HALO)]
        for j, sh in enumerate(SHIFTS[j0:j1]):
            win[pl.ds(HALO - sh, CH), pl.ds((j0 + j) * c4, c4)] = h[:, j * c4:(j + 1) * c4]

    def w2_stage(c, jobs):
        hs = h_v[pl.ds(pl.multiple_of(c * CH + HALO, HALO), CH), :].astype(BF16)
        y_v[chunk(c), :] = xn_v[chunk(c), :].astype(F32) + _dot_with_jobs(hs, w2_v[...], jobs)

    half = CH // RN // 2
    x_copy(0).wait()
    for job in norm_jobs(0):
        job()
    w1_left_copy.wait()
    w1_stage(0, [], 0, 2)
    x_copy(2).start()
    x_copy(1).wait()
    for job in norm_jobs(1):
        job()
    w2_copy.start()
    w1_right_copy.wait()
    w1_stage(0, [], 2, 4)

    @pl.loop(1, n_ch + 2)
    def _(c):
        @pl.when(c == 1)
        def _():
            for i in range(3, n_ch):
                x_copy(i).start()

        @pl.when(c == 2)
        def _():
            w2_copy.wait()
            for cp in late_copies + stage_copies(0, 0) + stage_copies(1, 1):
                cp.start()

        @pl.when(c + 1 < n_ch)
        def _():
            x_copy(c + 1).wait()

        jobs = norm_jobs(jnp.minimum(c + 1, n_ch - 1))

        @pl.when(c == 1)
        def _():
            for job in jobs[:half]:
                job()

        @pl.when(c >= 2)
        def _():
            w2_stage(c - 2, jobs[:half])

        @pl.when(c < n_ch)
        def _():
            w1_stage(c, jobs[half:])

    for job in norm3_jobs(0):
        job()

    for cp in late_copies:
        cp.wait()

    def repack_qkv(c, slot, w, blk, grp):
        st = (stq_v, stk_v, stv_v)[w]
        src = [pltpu.bitcast(st[slot, pl.ds((blk * 16 + d) * H + grp * 16, 16), :], U32)
               for d in range(16)]
        drow = pl.ds(pl.multiple_of(c * (d_ch // 2) + blk * 8, 8), 8)
        for j in range(2):
            words = [(a >> 16) | (b & np.uint32(0xFFFF0000)) if j
                     else (a & np.uint32(0xFFFF)) | (b << 16)
                     for a, b in zip(src[0::2], src[1::2])]
            for p, tile in enumerate(_transpose8(words)):
                wqkv_v[grp * 8 + p, drow, pl.ds((2 * w + j) * Dh, Dh)] = tile
        return wqkv_v[n_pair, pl.ds(pl.multiple_of(c * 8, 8), 8), pl.ds(0, 128)]

    def repack_o(c, slot, i):
        orow = pl.ds(pl.multiple_of(c * (o_ch // 2) + i * (RO // 2), RO // 2), RO // 2)
        wo_v[orow, :] = pltpu.bitcast(sto_v[slot, pl.ds(i * RO, RO), :], U32)
        return wo_v[pl.ds(pl.multiple_of(H * Dh // 2 + c * 8, 8), 8), pl.ds(0, 128)]

    @pl.loop(0, n_ch)
    def _(c):
        slot = c % 2
        for cp in stage_copies(c, slot):
            cp.wait()

        n_f = F // FC
        jobs = [functools.partial(repack_qkv, c, slot, w, blk, grp)
                for w in range(3) for blk in range(d_ch // 16) for grp in range(H // 16)]
        jobs += [functools.partial(repack_o, c, slot, i) for i in range(o_ch // RO)]
        jobs += norm3_jobs((c + 1) % n_ch)

        def share(k):
            return jobs[k * len(jobs) // (2 * n_f):(k + 1) * len(jobs) // (2 * n_f)]

        rows = chunk(c)
        u = {}
        for t in range(n_f + 1):
            if t < n_f:
                up = _dot(n3_v[rows, :], w3_v[:, pl.ds(t * FC, FC)])
                u[t] = _gelu(_jobs_before_use(up, share(max(2 * t - 1, 0)))).astype(BF16)
            if t >= 1:
                down = _dot(u.pop(t - 1), w4_v[pl.ds((t - 1) * FC, FC), :])
                down = _jobs_before_use(down, share(min(2 * t, 2 * n_f - 1)))
                y_v[rows, :] = y_v[rows, :] + down

        @pl.when(c + 2 < n_ch)
        def _():
            for cp in stage_copies(c + 2, slot):
                cp.start()

    L = M + SEG
    scale = Dh ** (-0.5)
    ri = lax.broadcasted_iota(jnp.int32, (2 * L, 2 * L), 0)
    ci = lax.broadcasted_iota(jnp.int32, (2 * L, 2 * L), 1)
    same_head = (ri >= L) == (ci >= L)
    rl = jnp.where(ri >= L, ri - L, ri)
    cl = jnp.where(ci >= L, ci - L, ci)
    visible = same_head & ((rl < M) | (rl >= cl))
    fill = jnp.where(same_head, np.float32(-1e9), np.float32(-np.inf))

    def heads_to_rows(y):
        return jnp.concatenate([y[:, :Dh], y[:, Dh:]], axis=0).astype(BF16)

    def segment(h, get_qkv, get_o):
        n_grp = n_pair // G
        qkv, probs, outs = {}, {}, {}
        acc = None
        for t in range(n_grp + 3):
            if t < n_grp:
                for p in range(t * G, (t + 1) * G):
                    y = get_qkv(p, _dot(h, pltpu.bitcast(wqkv_v[p], BF16)))
                    qkv[p] = [heads_to_rows(y[:, 2 * Dh * i:2 * Dh * (i + 1)]) for i in range(3)]
            if 0 <= t - 1 < n_grp:
                for p in range((t - 1) * G, t * G):
                    q, k, v = qkv.pop(p)
                    s = lax.dot_general(q, k, (((1,), (1,)), ((), ())),
                                        preferred_element_type=F32)
                    s = jnp.where(visible, s * scale, fill)
                    e = jnp.exp(s - jnp.max(s, axis=-1, keepdims=True))
                    l = jnp.sum(e, axis=-1, keepdims=True)
                    r = pl.reciprocal(l, approx=True)
                    probs[p] = (e.astype(BF16), v, r * (2.0 - l * r))
            if 0 <= t - 2 < n_grp:
                for p in range((t - 2) * G, (t - 1) * G):
                    e, v, r = probs.pop(p)
                    o = _dot(e, v) * r
                    outs[p] = get_o(p, jnp.concatenate([o[:L], o[L:]], axis=1)).astype(BF16)
            if 0 <= t - 3 < n_grp:
                p0 = (t - 3) * G
                o = jnp.concatenate([outs.pop(p) for p in range(p0, p0 + G)], axis=1)
                part = _dot(o, pltpu.bitcast(wo_v[pl.ds(p0 * Dh, G * Dh), :], BF16))
                acc = part if acc is None else acc + part
        return acc

    def two_segments(j, mem):
        rows = pl.ds(pl.multiple_of(j * (2 * SEG), 2 * SEG), 2 * SEG)
        xn = xn_v[rows, :].astype(F32)
        early_qkv, late_o = {}, {}

        def qkv_a(p, y):
            early_qkv[p] = y[L:]
            return y[:L]

        def o_a(p, o):
            late_o[p] = o[SEG:]
            return o[:SEG]

        def qkv_b(p, y):
            return jnp.concatenate([y[:M], early_qkv[p], y[M:]], axis=0)

        def o_b(p, o):
            return jnp.concatenate([o, late_o[p]], axis=0)

        acc_a = segment(jnp.concatenate([mem, xn[:L]], axis=0).astype(BF16), qkv_a, o_a)
        acc_b = segment(jnp.concatenate([acc_a[:M], xn[L:]], axis=0).astype(BF16), qkv_b, o_b)

        s = jnp.concatenate([acc_a[M:], acc_b[L:], acc_b[M:L]], axis=0)
        res = x_v[rows, :].astype(F32) + s * jax.nn.silu(y_v[rows, :])
        x_v[rows, :] = res.astype(x_v.dtype)
        pltpu.make_async_copy(x_v.at[rows], out_hbm.at[rows], o_sem.at[0]).start()
        return acc_b[:M]

    lax.fori_loop(0, S // (2 * SEG), two_segments, mem0_v[...].astype(F32))
    pltpu.make_async_copy(x_v, out_hbm, o_sem.at[0]).wait()


@functools.partial(jax.jit, static_argnames=("A_seg_len",))
def pallas_recurrent_scan__memory_aug_recurrent_mem_tr__mixer_s_mlp__prompt_kernel(
    A_x: jax.Array,
    A_mem0: jax.Array,
    A_Wq: jax.Array,
    A_Wk: jax.Array,
    A_Wv: jax.Array,
    A_Wo: jax.Array,
    A_seg_len: int,
    B_x: jax.Array,
    B_w1: jax.Array,
    B_w2: jax.Array,
    B_w3: jax.Array,
    B_w4: jax.Array,
):
    del B_x
    B, S, D = A_x.shape
    _, H, Dh = A_Wq.shape
    M = A_mem0.shape[1]
    F = B_w3.shape[1]
    SEG = int(A_seg_len)
    n_ch = S // CH
    d_ch = D // n_ch
    o_ch = (H * Dh) // n_ch
    assert B == 1 and S % CH == 0 and S % (2 * SEG) == 0 and F % FC == 0 and n_ch >= 4
    assert H % 16 == 0 and Dh == 128 and d_ch % 16 == 0 and M % 8 == 0 and SEG % 16 == 0

    any_spec = pl.BlockSpec(memory_space=pl.ANY)
    out = pl.pallas_call(
        functools.partial(_kernel, S=S, D=D, F=F, H=H, Dh=Dh, M=M, SEG=SEG),
        out_shape=jax.ShapeDtypeStruct((S, D), A_x.dtype),
        in_specs=[any_spec] * 10,
        out_specs=any_spec,
        scratch_shapes=[
            pltpu.VMEM((S, D), BF16),
            pltpu.VMEM((S, D), BF16),
            pltpu.VMEM((S + 16 * n_ch, D), BF16),
            pltpu.VMEM((S + 16 * n_ch, D), BF16),
            pltpu.VMEM((S + 2 * HALO, D), F32),
            pltpu.VMEM((S, D), F32),
            pltpu.VMEM((M, D), BF16),
            pltpu.VMEM((D, D), BF16),
            pltpu.VMEM((D, D), BF16),
            pltpu.VMEM((D, F), BF16),
            pltpu.VMEM((F, D), BF16),
            pltpu.VMEM((2, d_ch * H, Dh), BF16),
            pltpu.VMEM((2, d_ch * H, Dh), BF16),
            pltpu.VMEM((2, d_ch * H, Dh), BF16),
            pltpu.VMEM((2, o_ch, D), BF16),
            pltpu.VMEM((H // 2 + 1, D // 2, 6 * Dh), U32),
            pltpu.VMEM((H * Dh // 2 + 8 * n_ch, D), U32),
            pltpu.SemaphoreType.DMA((n_ch,)),
            pltpu.SemaphoreType.DMA((6,)),
            pltpu.SemaphoreType.DMA((8,)),
            pltpu.SemaphoreType.DMA((1,)),
        ],
        compiler_params=pltpu.CompilerParams(vmem_limit_bytes=120 * 1024 * 1024),
    )(
        A_x.reshape(S, D),
        A_mem0.reshape(M, D),
        A_Wq.reshape(D * H, Dh),
        A_Wk.reshape(D * H, Dh),
        A_Wv.reshape(D * H, Dh),
        A_Wo.reshape(H * Dh, D),
        B_w1, B_w2, B_w3, B_w4,
    )
    return out.reshape(B, S, D)
```
